```python
import jax
import jax.numpy as jnp

def _softmax(x, axis=-1):
    return jax.nn.softmax(x, axis=axis)
def _gelu(x):
    return jax.nn.gelu(x, approximate=True)
def _silu(x):
    return jax.nn.silu(x)
def _sigmoid(x):
    return jax.nn.sigmoid(x)
def _layernorm(x, axis=-1, eps=1e-5):
    m = jnp.mean(x, axis=axis, keepdims=True)
    v = jnp.var(x, axis=axis, keepdims=True)
    return (x - m) / jnp.sqrt(v + eps)
def _scatter_add(tgt, idx, src, axis=0):
    return tgt.at[idx].add(src)
def _segment_sum(src, seg, n):
    return jax.ops.segment_sum(src, seg, n)
class _Rng:
    def __init__(self, key):
        self._k = key
    def _next(self):
        self._k, sub = jax.random.split(self._k)
        return sub
    def normal(self, shape):
        return jax.random.normal(self._next(), shape, dtype=jnp.bfloat16)
    def randint(self, lo, hi, shape):
        return jax.random.randint(self._next(), shape, lo, hi, dtype=jnp.int32)
    def uniform(self, shape, lo=0.0, hi=1.0):
        return jax.random.uniform(self._next(), shape, jnp.bfloat16, lo, hi)
    def permutation(self, n):
        return jax.random.permutation(self._next(), n)


kernel_name = 'recurrent_scan__sliding_local_dilated__swiglu_ffn__prompt'

def setup_inputs():
    _rng = _Rng(jax.random.key(int.from_bytes(__import__("os").urandom(4), "little")))
    _w = (lambda a: (lambda t: t.astype(jnp.bfloat16) if jnp.issubdtype(t.dtype, jnp.floating) else t)(jnp.asarray(a)))
    def _A_setup():
        B, S, D = 1, 2048, 1024
        return {
            "x": _w((lambda *s: _rng.normal(s) * 0.05)(B, S, D)),
            "wqkv": _w((lambda *s: _rng.normal(s) * 0.05)(D, 3 * D)),
            "wo": _w((lambda *s: _rng.normal(s) * 0.05)(D, D)),
        }
    _A_in = _A_setup()

    def _B_setup():
        B, S, D, F = 1, 2048, 1024, 3584
        return {
            "x": _w((lambda *s: _rng.normal(s) * 0.05)(B, S, D)),
            "w_gate": _w((lambda *s: _rng.normal(s) * 0.05)(D, F)),
            "w_up": _w((lambda *s: _rng.normal(s) * 0.05)(D, F)),
            "w_down": _w((lambda *s: _rng.normal(s) * 0.05)(F, D)),
        }
    _B_in = _B_setup()

    return {
        "A_x": _A_in["x"],
        "A_wqkv": _A_in["wqkv"],
        "A_wo": _A_in["wo"],
        "B_x": _B_in["x"],
        "B_w_gate": _B_in["w_gate"],
        "B_w_up": _B_in["w_up"],
        "B_w_down": _B_in["w_down"],
    }

def reference(A_x, A_wqkv, A_wo, B_x, B_w_gate, B_w_up, B_w_down):
    def _A_ref(x, wqkv, wo):
        B, S, D = x.shape
        H = 32; Dh = D // H
        W, dil = 8, 2
        qkv = (lambda x, *d: x.transpose(*d))((x @ wqkv).reshape(B, S, 3, H, Dh), 2, 0, 3, 1, 4)
        q, k, v = qkv[0], qkv[1], qkv[2]
        scale = Dh ** -0.5
        pos = jnp.arange(S)
        off = jnp.arange(W) * dil
        idx = pos[:, None] - off[None, :]
        mask = idx >= 0
        idx_c = jnp.where(mask, idx, 0).reshape(-1)
        kg = k[:, :, idx_c, :].reshape(B, H, S, W, Dh)
        vg = v[:, :, idx_c, :].reshape(B, H, S, W, Dh)
        logits = jnp.einsum("bhsd,bhswd->bhsw", q, kg) * scale
        logits = jnp.where(mask[None, None, :, :], logits, -1e9)
        attn = _softmax(logits, axis=-1)
        o = jnp.einsum("bhsw,bhswd->bhsd", attn, vg)
        return (lambda x, *d: x.transpose(*d))(o, 0, 2, 1, 3).reshape(B, S, D) @ wo

    def _B_ref(x, w_gate, w_up, w_down):
        g = _silu(x @ w_gate)
        u = x @ w_up
        return (g * u) @ w_down

    x = A_x
    xn = _layernorm(x, axis=-1)
    s = _A_ref(xn, A_wqkv, A_wo)
    g = _silu(_B_ref(xn, B_w_gate, B_w_up, B_w_down))
    return x + s * g
```

```python
import functools
import math
import jax
import jax.numpy as jnp
import jax.experimental.pallas as pl
import jax.experimental.pallas.tpu as pltpu

F32 = jnp.float32
BF16 = jnp.bfloat16
U32 = jnp.uint32
HALO = 16
LANES = 128


def _butterfly(blocks):
    lane = jax.lax.broadcasted_iota(jnp.int32, blocks[0].shape, 1)
    for beta in (1, 2, 4):
        hi = (lane & (4 * beta)) != 0
        new = list(blocks)
        for j0 in range(8):
            if j0 & beta:
                continue
            j1 = j0 | beta
            new[j0] = jnp.where(hi, pltpu.roll(blocks[j1], 4 * beta, 1), blocks[j0])
            new[j1] = jnp.where(hi, blocks[j1], pltpu.roll(blocks[j0], LANES - 4 * beta, 1))
        blocks = new
    return blocks


def build(A_x, A_wqkv, A_wo, B_x, B_w_gate, B_w_up, B_w_down, TM=256, FC=512, WC=512, BR=16, late=1):
    B, S, D = A_x.shape
    F = B_w_gate.shape[1]
    H = 32
    Dh = D // H
    W, dil = 8, 2
    scale = Dh ** -0.5
    NB = D // LANES
    NT = S // TM
    RC = 16
    NWC = 3 * D // WC
    x2 = A_x.reshape(S, D)

    def kernel(x_hbm, wqkv_hbm, wo_hbm, wg_hbm, wu_hbm, wd_hbm, o_hbm,
               x_buf, xn_buf, wqkv, wo, wg, wu, wd, q_buf, k_buf, v_buf, a_buf, o_buf,
               x_sem, wc_sem, w_sem, o_sem):
        def x_cp(t):
            rows = pl.ds(pl.multiple_of(t * TM, TM), TM)
            return pltpu.make_async_copy(x_hbm.at[rows, :], x_buf.at[rows, :], x_sem.at[t])

        def o_cp(t):
            rows = pl.ds(pl.multiple_of(t * TM, TM), TM)
            return pltpu.make_async_copy(o_buf.at[rows, :], o_hbm.at[rows, :], o_sem.at[t])

        chunk_cols = [D * part + c for part in (2, 1, 0) for c in range(0, D, WC)]

        def wc_cp(n):
            cols = pl.ds(chunk_cols[n], WC)
            return pltpu.make_async_copy(wqkv_hbm.at[:, cols], wqkv.at[:, cols], wc_sem.at[n])

        big = [(wg_hbm, wg), (wu_hbm, wu), (wd_hbm, wd), (wo_hbm, wo)]

        def w_cp(n):
            return pltpu.make_async_copy(big[n][0], big[n][1], w_sem.at[n])

        def start_rest():
            for t in range(2, NT):
                x_cp(t).start()
            for n in range(len(big)):
                w_cp(n).start()

        def layernorm(t):
            rows = pl.ds(pl.multiple_of(t * TM, TM), TM)
            x = x_buf[rows, :].astype(F32)
            m = jnp.mean(x, axis=-1, keepdims=True)
            xc = x - m
            var = jnp.mean(xc * xc, axis=-1, keepdims=True)
            xn_buf[rows, :] = (xc * jax.lax.rsqrt(var + 1e-5)).astype(BF16)

        def store_permuted(y, dst, t):
            for r in range(0, TM, BR):
                yi = pltpu.bitcast(y[r:r + BR, :].astype(BF16), U32)
                blocks = _butterfly([yi[:, LANES * j:LANES * (j + 1)] for j in range(NB)])
                for j in range(NB):
                    dst[j, pl.ds(pl.multiple_of(t * TM + HALO + r, 8), BR), :] = (
                        pltpu.bitcast(blocks[j], BF16).astype(F32))

        def phase_a(t, first):
            rows = pl.ds(pl.multiple_of(t * TM, TM), TM)
            parts = []
            for n in range(NWC):
                if first:
                    wc_cp(n).wait()
                    if n == late:
                        start_rest()
                c0 = chunk_cols[n]
                parts.append(jnp.dot(xn_buf[rows, :], wqkv[:, c0:c0 + WC], preferred_element_type=F32))
                if (n + 1) * WC % D == 0:
                    y = jnp.concatenate(parts, axis=1) if len(parts) > 1 else parts[0]
                    parts = []
                    which = (n + 1) * WC // D
                    if which == 1:
                        store_permuted(y, v_buf, t)
                    elif which == 2:
                        store_permuted(y, k_buf, t)
                    else:
                        q_buf[pl.ds(pl.multiple_of(t * (TM // 2), TM // 2), TM // 2), :] = (
                            pltpu.bitcast(y.astype(BF16), U32))
            if first:
                x_cp(1).wait()
                layernorm(1)
            else:
                layernorm(jnp.minimum(t + 1, NT - 1))

        lane = jax.lax.broadcasted_iota(jnp.int32, (RC, LANES), 1)
        odd = (lane & 1) == 1
        hi2 = (lane & 2) == 2
        rowi = jax.lax.broadcasted_iota(jnp.int32, (RC, LANES), 0)
        cexp = scale * math.log2(math.e)

        def attn_chunk(t, r0):
            qi = q_buf[pl.ds(pl.multiple_of(t * (TM // 2) + r0 // 2, 8), RC // 2), :]
            qb = _butterfly([qi[:, LANES * j:LANES * (j + 1)] for j in range(NB)])
            qs = [pltpu.bitcast(b, BF16).astype(F32) for b in qb]
            base = pl.multiple_of(t * TM, TM) + (HALO + r0)
            logits = []
            for w in range(W):
                acc = qs[0] * k_buf[0, pl.ds(base - dil * w, RC), :]
                for j in range(1, NB):
                    acc = acc + qs[j] * k_buf[j, pl.ds(base - dil * w, RC), :]
                acc = acc + jnp.where(odd, pltpu.roll(acc, 1, 1), pltpu.roll(acc, LANES - 1, 1))
                acc = acc + jnp.where(hi2, pltpu.roll(acc, 2, 1), pltpu.roll(acc, LANES - 2, 1))
                if w > 0 and r0 < dil * w:
                    pos = rowi + (t * TM + r0 - dil * w)
                    acc = jnp.where(pos >= 0, acc, -1e9 / scale)
                logits.append(acc)
            mx = logits[0]
            for w in range(1, W):
                mx = jnp.maximum(mx, logits[w])
            ps = [jnp.exp2((l - mx) * cexp) for l in logits]
            den = ps[0]
            for w in range(1, W):
                den = den + ps[w]
            inv = 1.0 / den
            ps = [p * inv for p in ps]
            outs = []
            for j in range(NB):
                o = ps[0] * v_buf[j, pl.ds(base, RC), :]
                for w in range(1, W):
                    o = o + ps[w] * v_buf[j, pl.ds(base - dil * w, RC), :]
                outs.append(pltpu.bitcast(o.astype(BF16), U32))
            ob = _butterfly(outs)
            for j in range(NB):
                a_buf[r0 // 2:(r0 + RC) // 2, LANES * j:LANES * (j + 1)] = ob[j]

        def phase_b(t):
            rows = pl.ds(pl.multiple_of(t * TM, TM), TM)
            xn = xn_buf[rows, :]
            for r0 in range(0, TM, RC):
                attn_chunk(t, r0)
            acc = None
            for c in range(F // FC):
                g = jnp.dot(xn, wg[:, c * FC:(c + 1) * FC], preferred_element_type=F32)
                u = jnp.dot(xn, wu[:, c * FC:(c + 1) * FC], preferred_element_type=F32)
                h = (g * jax.nn.sigmoid(g) * u).astype(BF16)
                d = jnp.dot(h, wd[c * FC:(c + 1) * FC, :], preferred_element_type=F32)
                acc = d if acc is None else acc + d
            gate = acc * jax.nn.sigmoid(acc)
            s = jnp.dot(pltpu.bitcast(a_buf[...], BF16), wo[...], preferred_element_type=F32)
            o_buf[rows, :] = (x_buf[rows, :].astype(F32) + s * gate).astype(BF16)
            o_cp(t).start()

        x_cp(0).start()
        for n in range(NWC):
            wc_cp(n).start()
        x_cp(1).start()
        k_buf[:, 0:HALO, :] = jnp.zeros((NB, HALO, LANES), F32)
        v_buf[:, 0:HALO, :] = jnp.zeros((NB, HALO, LANES), F32)
        x_cp(0).wait()
        layernorm(0)
        phase_a(0, True)

        def a_body(t, c):
            @pl.when(t + 1 < NT)
            def _():
                x_cp(t + 1).wait()
            phase_a(t, False)
            return c
        jax.lax.fori_loop(1, NT, a_body, 0)

        for n in range(len(big)):
            w_cp(n).wait()

        def b_body(t, c):
            phase_b(t)
            return c
        jax.lax.fori_loop(0, NT, b_body, 0)
        for t in range(NT):
            o_cp(t).wait()

    anyspec = pl.BlockSpec(memory_space=pl.ANY)
    out = pl.pallas_call(
        kernel,
        in_specs=[anyspec] * 6,
        out_specs=anyspec,
        out_shape=jax.ShapeDtypeStruct((S, D), A_x.dtype),
        scratch_shapes=[
            pltpu.VMEM((S, D), BF16), pltpu.VMEM((S, D), BF16),
            pltpu.VMEM((D, 3 * D), BF16), pltpu.VMEM((D, D), BF16),
            pltpu.VMEM((D, F), BF16), pltpu.VMEM((D, F), BF16), pltpu.VMEM((F, D), BF16),
            pltpu.VMEM((S // 2, D), U32),
            pltpu.VMEM((NB, S + HALO, LANES), F32), pltpu.VMEM((NB, S + HALO, LANES), F32),
            pltpu.VMEM((TM // 2, D), U32), pltpu.VMEM((S, D), BF16),
            pltpu.SemaphoreType.DMA((NT,)), pltpu.SemaphoreType.DMA((NWC,)),
            pltpu.SemaphoreType.DMA((4,)), pltpu.SemaphoreType.DMA((NT,)),
        ],
        compiler_params=pltpu.CompilerParams(vmem_limit_bytes=110 * 1024 * 1024),
    )(x2, A_wqkv, A_wo, B_w_gate, B_w_up, B_w_down)
    return out.reshape(B, S, D)


@jax.jit
def pallas_recurrent_scan__sliding_local_dilated__swiglu_ffn__prompt_kernel(A_x, A_wqkv, A_wo, B_x, B_w_gate, B_w_up, B_w_down):
    return build(A_x, A_wqkv, A_wo, B_x, B_w_gate, B_w_up, B_w_down)
```

```python
import contextlib
import math
import jax
import jax.numpy as jnp
import jax.experimental.pallas as pl
import jax.experimental.pallas.tpu as pltpu

F32 = jnp.float32
BF16 = jnp.bfloat16
U32 = jnp.uint32
HALO = 16
LANES = 128


def _butterfly(blocks):
    lane = jax.lax.broadcasted_iota(jnp.int32, blocks[0].shape, 1)
    for beta in (1, 2, 4):
        hi = (lane & (4 * beta)) != 0
        new = list(blocks)
        for j0 in range(8):
            if j0 & beta:
                continue
            j1 = j0 | beta
            new[j0] = jnp.where(hi, pltpu.roll(blocks[j1], 4 * beta, 1), blocks[j0])
            new[j1] = jnp.where(hi, blocks[j1], pltpu.roll(blocks[j0], LANES - 4 * beta, 1))
        blocks = new
    return blocks


def _opaque_zero(v):
    s = jnp.uint32(16)
    return jax.lax.shift_right_logical(jax.lax.shift_right_logical(v, s), s)


def _fzero(v):
    return pltpu.bitcast(_opaque_zero(pltpu.bitcast(v, U32)), F32)


def _silu(x):
    hx = 0.5 * x
    return hx * (1.0 + jnp.tanh(hx))


def _pack(y):
    return pltpu.bitcast(y.astype(BF16), U32)


def build(A_x, A_wqkv, A_wo, B_x, B_w_gate, B_w_up, B_w_down, TM=256, FC=512,
          chunks=(256, 256, 512, 512, 512), chain=1, pchain=2, lng=32, lnchain=1, opaque=True, ser=1, serv=1, scopes=False):
    scope = jax.named_scope if scopes else (lambda name: contextlib.nullcontext())
    B, S, D = A_x.shape
    F = B_w_gate.shape[1]
    H = 32
    Dh = D // H
    W, dil = 8, 2
    scale = Dh ** -0.5
    NB = D // LANES
    NT = S // TM
    RC = 16
    TH = TM // 2
    NWC = len(chunks)
    assert sum(chunks) == 2 * D
    chunk_off = [sum(chunks[:n]) for n in range(NWC)]
    x2 = A_x.reshape(S, D)

    def kernel(x_hbm, wqkv_hbm, wo_hbm, wg_hbm, wu_hbm, wd_hbm, o_hbm,
               x_buf, xn_buf, wqkv, wo, wg, wu, wd, kv_raw, q_buf, k_buf, v_buf, a_buf, o_buf, off_tab,
               x_sem, wc_sem, w_sem, o_sem):
        def tile_rows(t):
            return pl.ds(pl.multiple_of(t * TM, TM), TM)

        def half_rows(t):
            return pl.ds(pl.multiple_of(t * TH, TH), TH)

        def x_cp(t):
            return pltpu.make_async_copy(x_hbm.at[tile_rows(t), :], x_buf.at[tile_rows(t), :], x_sem.at[t])

        def o_cp(t):
            return pltpu.make_async_copy(o_buf.at[tile_rows(t), :], o_hbm.at[tile_rows(t), :], o_sem.at[t])

        def wc_cp(n):
            cols = pl.ds(D + chunk_off[n], chunks[n])
            return pltpu.make_async_copy(wqkv_hbm.at[:, cols], wqkv.at[:, cols], wc_sem.at[n])

        big = [(wqkv_hbm.at[:, 0:D], wqkv.at[:, 0:D]), (wg_hbm, wg), (wu_hbm, wu), (wd_hbm, wd), (wo_hbm, wo)]

        def w_cp(n):
            return pltpu.make_async_copy(big[n][0], big[n][1], w_sem.at[n])

        def layernorm(t, nchain=0):
            deps = []
            step = lng if nchain else TM
            for r in range(0, TM, step):
                rows = pl.ds(pl.multiple_of(t * TM + r, step), step)
                x = x_buf[rows, :].astype(F32)
                m = jnp.mean(x, axis=-1, keepdims=True)
                if nchain and len(deps) >= nchain:
                    m = m + pltpu.bitcast(_opaque_zero(deps[-nchain]), F32)
                xc = x - m
                var = jnp.mean(xc * xc, axis=-1, keepdims=True)
                xn = xc * jax.lax.rsqrt(var + 1e-5)
                if nchain:
                    deps.append(pltpu.bitcast(xn[:, D - 1:D], U32))
                xn_buf[rows, :] = xn.astype(BF16)

        def phase_a0():
            for n in range(NWC):
                with scope(f"wcwait{n}"):
                    wc_cp(n).wait()
                if n == 0:
                    for m in range(len(big)):
                        w_cp(m).start(priority=1)
                if n == NWC - 1:
                    for tt in range(2, NT):
                        x_cp(tt).start()
                    x_cp(1).wait()
                    layernorm(1, lnchain)
                c0, cw = chunk_off[n], chunks[n]
                kv_raw[0:TH, c0:c0 + cw] = _pack(
                    jnp.dot(xn_buf[0:TM, :], wqkv[:, D + c0:D + c0 + cw], preferred_element_type=F32))

        def phase_a(t):
            kv_raw[half_rows(t), :] = _pack(
                jnp.dot(xn_buf[tile_rows(t), :], wqkv[:, D:3 * D], preferred_element_type=F32))
            layernorm(jnp.minimum(t + 1, NT - 1), lnchain)

        def permute_kv(t):
            deps = []
            for r in range(0, TM, 16):
                for part, dst in ((0, k_buf), (1, v_buf)):
                    src_rows = pl.ds(pl.multiple_of(t * TH + r // 2, 8), 8)
                    blocks = [kv_raw[src_rows, part * D + LANES * j:part * D + LANES * (j + 1)] for j in range(NB)]
                    if len(deps) >= pchain:
                        zero = _opaque_zero(deps[-pchain])
                        blocks = [b | zero for b in blocks]
                    blocks = _butterfly(blocks)
                    deps.append(blocks[NB - 1])
                    for j in range(NB):
                        dst[j, pl.ds(pl.multiple_of(t * TM + HALO + r, 8), 16), :] = (
                            pltpu.bitcast(blocks[j], BF16).astype(F32))
            dep = deps[-1]
            for d in deps[-pchain:-1]:
                dep = dep | d
            return dep

        lane = jax.lax.broadcasted_iota(jnp.int32, (RC, LANES), 1)
        odd = (lane & 1) == 1
        hi2 = (lane & 2) == 2
        rowi = jax.lax.broadcasted_iota(jnp.int32, (RC, LANES), 0)
        cexp = scale * math.log2(math.e)

        def attn_chunk(t, row0, r0, dep):
            zero = _opaque_zero(dep)
            qb = _butterfly([q_buf[r0 // 2:(r0 + RC) // 2, LANES * j:LANES * (j + 1)] | zero for j in range(NB)])
            qs = [pltpu.bitcast(b, BF16).astype(F32) for b in qb]
            base = row0 + (HALO + r0)
            logits = []
            raws = []
            for w in range(W):
                acc = qs[0] * k_buf[0, pl.ds(base - dil * w, RC), :]
                if ser and w >= ser:
                    acc = acc + _fzero(raws[-ser])
                for j in range(1, NB):
                    acc = acc + qs[j] * k_buf[j, pl.ds(base - dil * w, RC), :]
                raws.append(acc)
                acc = acc + jnp.where(odd, pltpu.roll(acc, 1, 1), pltpu.roll(acc, LANES - 1, 1))
                acc = acc + jnp.where(hi2, pltpu.roll(acc, 2, 1), pltpu.roll(acc, LANES - 2, 1))
                if w > 0 and r0 < dil * w:
                    pos = rowi + (t * TM + r0 - dil * w)
                    acc = jnp.where(pos >= 0, acc, -1e9 / scale)
                logits.append(acc)
            mx = logits[0]
            for w in range(1, W):
                mx = jnp.maximum(mx, logits[w])
            ps = [jnp.exp2((l - mx) * cexp) for l in logits]
            den = ps[0]
            for w in range(1, W):
                den = den + ps[w]
            inv = 1.0 / den
            ps = [p * inv for p in ps]
            outs = []
            raws = []
            for j in range(NB):
                o = ps[0] * v_buf[j, pl.ds(base, RC), :]
                if serv and j >= serv:
                    o = o + _fzero(raws[-serv])
                for w in range(1, W):
                    o = o + ps[w] * v_buf[j, pl.ds(base - dil * w, RC), :]
                raws.append(o)
                outs.append(_pack(o))
            ob = _butterfly(outs)
            for j in range(NB):
                a_buf[r0 // 2:(r0 + RC) // 2, LANES * j:LANES * (j + 1)] = ob[j]
            return ob[NB - 1]

        def phase_b(t):
            rows = tile_rows(t)
            xn = xn_buf[rows, :]
            q_buf[...] = _pack(jnp.dot(xn, wqkv[:, 0:D], preferred_element_type=F32))
            deps = [permute_kv(t)] * chain
            row0 = off_tab[t] if opaque else t * TM
            for r0 in range(0, TM, RC):
                deps.append(attn_chunk(t, row0, r0, deps[-chain]))
            acc = None
            for c in range(F // FC):
                g = jnp.dot(xn, wg[:, c * FC:(c + 1) * FC], preferred_element_type=F32)
                u = jnp.dot(xn, wu[:, c * FC:(c + 1) * FC], preferred_element_type=F32)
                h = (_silu(g) * u).astype(BF16)
                d = jnp.dot(h, wd[c * FC:(c + 1) * FC, :], preferred_element_type=F32)
                acc = d if acc is None else acc + d
            gate = _silu(acc)
            s = jnp.dot(pltpu.bitcast(a_buf[...], BF16), wo[...], preferred_element_type=F32)
            o_buf[rows, :] = (x_buf[rows, :].astype(F32) + s * gate).astype(BF16)
            o_cp(t).start()

        x_cp(0).start()
        wc_cp(0).start(priority=1)
        for t in range(NT):
            off_tab[t] = t * TM
        k_buf[:, 0:HALO, :] = jnp.zeros((NB, HALO, LANES), F32)
        v_buf[:, 0:HALO, :] = jnp.zeros((NB, HALO, LANES), F32)
        with scope("x0wait"):
            x_cp(0).wait()
        for n in range(1, NWC):
            wc_cp(n).start(priority=1)
        x_cp(1).start(priority=1)
        with scope("ln0"):
            layernorm(0)
        phase_a0()

        def a_body(t, c):
            @pl.when(t + 1 < NT)
            def _():
                x_cp(t + 1).wait()
            with scope("A"):
                phase_a(t)
            return c
        jax.lax.fori_loop(1, NT, a_body, 0)

        with scope("bigwait"):
            for n in range(len(big)):
                w_cp(n).wait()

        def b_body(t, c):
            with scope("B"):
                phase_b(t)
            return c
        jax.lax.fori_loop(0, NT, b_body, 0)
        with scope("owait"):
            for t in range(NT):
                o_cp(t).wait()

    anyspec = pl.BlockSpec(memory_space=pl.ANY)
    out = pl.pallas_call(
        kernel,
        in_specs=[anyspec] * 6,
        out_specs=anyspec,
        out_shape=jax.ShapeDtypeStruct((S, D), A_x.dtype),
        scratch_shapes=[
            pltpu.VMEM((S, D), BF16), pltpu.VMEM((S, D), BF16),
            pltpu.VMEM((D, 3 * D), BF16), pltpu.VMEM((D, D), BF16),
            pltpu.VMEM((D, F), BF16), pltpu.VMEM((D, F), BF16), pltpu.VMEM((F, D), BF16),
            pltpu.VMEM((S // 2, 2 * D), U32), pltpu.VMEM((TH, D), U32),
            pltpu.VMEM((NB, S + HALO, LANES), F32), pltpu.VMEM((NB, S + HALO, LANES), F32),
            pltpu.VMEM((TH, D), U32), pltpu.VMEM((S, D), BF16), pltpu.SMEM((NT,), jnp.int32),
            pltpu.SemaphoreType.DMA((NT,)), pltpu.SemaphoreType.DMA((NWC,)),
            pltpu.SemaphoreType.DMA((5,)), pltpu.SemaphoreType.DMA((NT,)),
        ],
        compiler_params=pltpu.CompilerParams(vmem_limit_bytes=110 * 1024 * 1024),
    )(x2, A_wqkv, A_wo, B_w_gate, B_w_up, B_w_down)
    return out.reshape(B, S, D)


@jax.jit
def pallas_recurrent_scan__sliding_local_dilated__swiglu_ffn__prompt_kernel(A_x, A_wqkv, A_wo, B_x, B_w_gate, B_w_up, B_w_down):
    return build(A_x, A_wqkv, A_wo, B_x, B_w_gate, B_w_up, B_w_down)
```

```python
import contextlib
import math
import jax
import jax.numpy as jnp
import jax.experimental.pallas as pl
import jax.experimental.pallas.tpu as pltpu

F32 = jnp.float32
BF16 = jnp.bfloat16
U32 = jnp.uint32
HALO = 16
LANES = 128


def _butterfly(blocks):
    lane = jax.lax.broadcasted_iota(jnp.int32, blocks[0].shape, 1)
    for beta in (1, 2, 4):
        hi = (lane & (4 * beta)) != 0
        new = list(blocks)
        for j0 in range(8):
            if j0 & beta:
                continue
            j1 = j0 | beta
            new[j0] = jnp.where(hi, pltpu.roll(blocks[j1], 4 * beta, 1), blocks[j0])
            new[j1] = jnp.where(hi, blocks[j1], pltpu.roll(blocks[j0], LANES - 4 * beta, 1))
        blocks = new
    return blocks


def _opaque_zero(v):
    s = jnp.uint32(16)
    return jax.lax.shift_right_logical(jax.lax.shift_right_logical(v, s), s)


def _fzero(v):
    return pltpu.bitcast(_opaque_zero(pltpu.bitcast(v, U32)), F32)


def _silu(x):
    hx = 0.5 * x
    return hx * (1.0 + jnp.tanh(hx))


def _tree(op, xs):
    xs = list(xs)
    while len(xs) > 1:
        xs = [op(xs[i], xs[i + 1]) if i + 1 < len(xs) else xs[i] for i in range(0, len(xs), 2)]
    return xs[0]


def _pack(y):
    return pltpu.bitcast(y.astype(BF16), U32)


def build(A_x, A_wqkv, A_wo, B_x, B_w_gate, B_w_up, B_w_down, TM=256, FC=512,
          chunks=(128, 256, 256, 384, 384, 384, 256), chain=1, pchain=2, lng=32, lnchain=1, opaque=True, ser=1, serv=1, SR=16, split=None, ln1=None, bigat=5, ln1chain=4, nochk=True, osplit=(768, 256), midk='pv', nextk='end', fastinv=True, postnorm=True, scopes=False):
    scope = jax.named_scope if scopes else (lambda name: contextlib.nullcontext())
    B, S, D = A_x.shape
    F = B_w_gate.shape[1]
    H = 32
    Dh = D // H
    W, dil = 8, 2
    scale = Dh ** -0.5
    NB = D // LANES
    NT = S // TM
    RC = 16
    TH = TM // 2
    NWC = len(chunks)
    assert sum(chunks) == 2 * D
    nsplit = NWC if split is None else split
    nln1 = NWC - 1 if ln1 is None else ln1
    chunk_off = [sum(chunks[:n]) for n in range(NWC)]
    x2 = A_x.reshape(S, D)

    def kernel(x_hbm, wqkv_hbm, wo_hbm, wg_hbm, wu_hbm, wd_hbm, o_hbm,
               x_buf, xn_buf, wqkv, wo, wg, wu, wd, kv_raw, q_buf, k_buf, v_buf, a_buf, o_buf, off_tab,
               x_sem, wc_sem, w_sem, o_sem):
        def tile_rows(t):
            return pl.ds(pl.multiple_of(t * TM, TM), TM)

        def half_rows(t):
            return pl.ds(pl.multiple_of(t * TH, TH), TH)

        def x_cp(t):
            return pltpu.make_async_copy(x_hbm.at[tile_rows(t), :], x_buf.at[tile_rows(t), :], x_sem.at[t])

        def o_cp(t, p):
            cols = pl.ds(sum(osplit[:p]), osplit[p])
            return pltpu.make_async_copy(o_buf.at[tile_rows(t), cols], o_hbm.at[tile_rows(t), cols],
                                         o_sem.at[t * len(osplit) + p])

        def wc_cp(n):
            cols = pl.ds(D + chunk_off[n], chunks[n])
            return pltpu.make_async_copy(wqkv_hbm.at[:, cols], wqkv.at[:, cols], wc_sem.at[n])

        big = [(wqkv_hbm.at[:, 0:D], wqkv.at[:, 0:D]), (wg_hbm, wg), (wu_hbm, wu), (wd_hbm, wd), (wo_hbm, wo)]

        def w_cp(n):
            return pltpu.make_async_copy(big[n][0], big[n][1], w_sem.at[n])

        def layernorm(t, nchain=0):
            deps = []
            step = lng if nchain else TM
            for r in range(0, TM, step):
                rows = pl.ds(pl.multiple_of(t * TM + r, step), step)
                x = x_buf[rows, :].astype(F32)
                m = jnp.mean(x, axis=-1, keepdims=True)
                if nchain and len(deps) >= nchain:
                    m = m + pltpu.bitcast(_opaque_zero(deps[-nchain]), F32)
                xc = x - m
                var = jnp.mean(xc * xc, axis=-1, keepdims=True)
                xn = xc * jax.lax.rsqrt(var + 1e-5)
                if nchain:
                    deps.append(pltpu.bitcast(xn[:, D - 1:D], U32))
                xn_buf[rows, :] = xn.astype(BF16)

        def phase_a0():
            for n in range(NWC):
                with scope(f"wcwait{n}"):
                    wc_cp(n).wait()
                if n == 0:
                    x_cp(1).start(priority=1)
                if n == 1:
                    for m in range(nsplit, NWC):
                        wc_cp(m).start(priority=1)
                if n == bigat:
                    for m in range(len(big)):
                        w_cp(m).start(priority=1)
                if n == NWC - 1:
                    for tt in range(2, NT):
                        x_cp(tt).start()
                if n == nln1:
                    with scope("x1wait"):
                        x_cp(1).wait()
                    layernorm(1, ln1chain)
                c0, cw = chunk_off[n], chunks[n]
                kv_raw[0:TH, c0:c0 + cw] = _pack(
                    jnp.dot(xn_buf[0:TM, :], wqkv[:, D + c0:D + c0 + cw], preferred_element_type=F32))

        def phase_a(t):
            kv_raw[half_rows(t), :] = _pack(
                jnp.dot(xn_buf[tile_rows(t), :], wqkv[:, D:3 * D], preferred_element_type=F32))
            layernorm(jnp.minimum(t + 1, NT - 1), lnchain)

        def permute_kv(t):
            deps = []
            for r in range(0, TM, 16):
                for part, dst in ((0, k_buf), (1, v_buf)):
                    src_rows = pl.ds(pl.multiple_of(t * TH + r // 2, 8), 8)
                    blocks = [kv_raw[src_rows, part * D + LANES * j:part * D + LANES * (j + 1)] for j in range(NB)]
                    if len(deps) >= pchain:
                        zero = _opaque_zero(deps[-pchain])
                        blocks = [b | zero for b in blocks]
                    blocks = _butterfly(blocks)
                    deps.append(blocks[NB - 1])
                    for j in range(NB):
                        dst[j, pl.ds(pl.multiple_of(t * TM + HALO + r, 8), 16), :] = (
                            pltpu.bitcast(blocks[j], BF16).astype(F32))
            dep = deps[-1]
            for d in deps[-pchain:-1]:
                dep = dep | d
            return dep

        lane = jax.lax.broadcasted_iota(jnp.int32, (SR, LANES), 1)
        odd = (lane & 1) == 1
        hi2 = (lane & 2) == 2
        rowi = jax.lax.broadcasted_iota(jnp.int32, (SR, LANES), 0)
        cexp = scale * math.log2(math.e)

        def attn_rows(t, row0, r0, qs, dep):
            base = row0 + (HALO + r0)
            logits = []
            raws = [dep] * ser
            for w in range(W):
                acc = qs[0] * k_buf[0, pl.ds(base - dil * w, SR), :]
                if raws[-ser] is not None:
                    acc = acc + _fzero(raws[-ser])
                for j in range(1, NB):
                    acc = acc + qs[j] * k_buf[j, pl.ds(base - dil * w, SR), :]
                raws.append(acc)
                acc = acc + jnp.where(odd, pltpu.roll(acc, 1, 1), pltpu.roll(acc, LANES - 1, 1))
                acc = acc + jnp.where(hi2, pltpu.roll(acc, 2, 1), pltpu.roll(acc, LANES - 2, 1))
                if w > 0 and r0 < dil * w:
                    pos = rowi + (t * TM + r0 - dil * w)
                    acc = jnp.where(pos >= 0, acc, -1e9 / scale)
                logits.append(acc)
            mx = _tree(jnp.maximum, logits)
            ps = [jnp.exp2((l - mx) * cexp) for l in logits]
            den = _tree(jnp.add, ps)
            if fastinv:
                r = pl.reciprocal(den, approx=True)
                inv = r * (2.0 - den * r)
            else:
                inv = 1.0 / den
            if not postnorm:
                ps = [p * inv for p in ps]
            raws = []
            outs = []
            for j in range(NB):
                o = ps[0] * v_buf[j, pl.ds(base, SR), :]
                if serv and j >= serv:
                    o = o + _fzero(raws[-serv])
                for w in range(1, W):
                    o = o + ps[w] * v_buf[j, pl.ds(base - dil * w, SR), :]
                raws.append(o)
                outs.append(o * inv if postnorm else o)
            mid = {"sm": inv, "pv": raws[-1], "qk": logits[-1]}[midk]
            return outs, mid

        def attn_chunk(t, row0, r0, dep):
            zero = _opaque_zero(dep)
            qb = _butterfly([q_buf[r0 // 2:(r0 + RC) // 2, LANES * j:LANES * (j + 1)] | zero for j in range(NB)])
            qs = [pltpu.bitcast(b, BF16).astype(F32) for b in qb]
            parts = []
            mid = None
            for h in range(0, RC, SR):
                o, mid = attn_rows(t, row0, r0 + h, [q[h:h + SR] for q in qs], mid)
                parts.append(o)
            ob = _butterfly([_pack(jnp.concatenate([p[j] for p in parts], axis=0)) for j in range(NB)])
            for j in range(NB):
                a_buf[r0 // 2:(r0 + RC) // 2, LANES * j:LANES * (j + 1)] = ob[j]
            return ob[NB - 1] if nextk == "end" else pltpu.bitcast(mid[0:8], U32)

        def phase_b(t):
            rows = tile_rows(t)
            xn = xn_buf[rows, :]
            q_buf[...] = _pack(jnp.dot(xn, wqkv[:, 0:D], preferred_element_type=F32))
            deps = [permute_kv(t)] * chain
            row0 = off_tab[t] if opaque else t * TM
            for r0 in range(0, TM, RC):
                deps.append(attn_chunk(t, row0, r0, deps[-chain]))
            acc = None
            for c in range(F // FC):
                g = jnp.dot(xn, wg[:, c * FC:(c + 1) * FC], preferred_element_type=F32)
                u = jnp.dot(xn, wu[:, c * FC:(c + 1) * FC], preferred_element_type=F32)
                h = (_silu(g) * u).astype(BF16)
                d = jnp.dot(h, wd[c * FC:(c + 1) * FC, :], preferred_element_type=F32)
                acc = d if acc is None else acc + d
            a = pltpu.bitcast(a_buf[...], BF16)
            for p in range(len(osplit)):
                c0, c1 = sum(osplit[:p]), sum(osplit[:p + 1])
                s = jnp.dot(a, wo[:, c0:c1], preferred_element_type=F32)
                o_buf[rows, c0:c1] = (x_buf[rows, c0:c1].astype(F32) + s * _silu(acc[:, c0:c1])).astype(BF16)
                o_cp(t, p).start()

        x_cp(0).start()
        wc_cp(0).start(priority=1)
        for t in range(NT):
            off_tab[t] = t * TM
        k_buf[:, 0:HALO, :] = jnp.zeros((NB, HALO, LANES), F32)
        v_buf[:, 0:HALO, :] = jnp.zeros((NB, HALO, LANES), F32)
        with scope("x0wait"):
            x_cp(0).wait()
        for n in range(1, nsplit):
            wc_cp(n).start(priority=1)
        with scope("ln0"):
            layernorm(0)
        phase_a0()

        def a_body(t, c):
            @pl.when(t + 1 < NT)
            def _():
                x_cp(t + 1).wait()
            with scope("A"):
                phase_a(t)
            return c
        jax.lax.fori_loop(1, NT, a_body, 0)

        with scope("bigwait"):
            for n in range(len(big)):
                w_cp(n).wait()

        def b_body(t, c):
            with scope("B"):
                phase_b(t)
            return c
        jax.lax.fori_loop(0, NT, b_body, 0)
        with scope("owait"):
            for t in range(NT):
                for p in range(len(osplit)):
                    o_cp(t, p).wait()

    anyspec = pl.BlockSpec(memory_space=pl.ANY)
    out = pl.pallas_call(
        kernel,
        in_specs=[anyspec] * 6,
        out_specs=anyspec,
        out_shape=jax.ShapeDtypeStruct((S, D), A_x.dtype),
        scratch_shapes=[
            pltpu.VMEM((S, D), BF16), pltpu.VMEM((S, D), BF16),
            pltpu.VMEM((D, 3 * D), BF16), pltpu.VMEM((D, D), BF16),
            pltpu.VMEM((D, F), BF16), pltpu.VMEM((D, F), BF16), pltpu.VMEM((F, D), BF16),
            pltpu.VMEM((S // 2, 2 * D), U32), pltpu.VMEM((TH, D), U32),
            pltpu.VMEM((NB, S + HALO, LANES), F32), pltpu.VMEM((NB, S + HALO, LANES), F32),
            pltpu.VMEM((TH, D), U32), pltpu.VMEM((S, D), BF16), pltpu.SMEM((NT,), jnp.int32),
            pltpu.SemaphoreType.DMA((NT,)), pltpu.SemaphoreType.DMA((NWC,)),
            pltpu.SemaphoreType.DMA((5,)), pltpu.SemaphoreType.DMA((NT * len(osplit),)),
        ],
        compiler_params=pltpu.CompilerParams(vmem_limit_bytes=110 * 1024 * 1024, disable_bounds_checks=nochk,
                                             disable_semaphore_checks=nochk),
    )(x2, A_wqkv, A_wo, B_w_gate, B_w_up, B_w_down)
    return out.reshape(B, S, D)


@jax.jit
def pallas_recurrent_scan__sliding_local_dilated__swiglu_ffn__prompt_kernel(A_x, A_wqkv, A_wo, B_x, B_w_gate, B_w_up, B_w_down):
    return build(A_x, A_wqkv, A_wo, B_x, B_w_gate, B_w_up, B_w_down)
```

```python
import contextlib
import math
import jax
import jax.numpy as jnp
import jax.experimental.pallas as pl
import jax.experimental.pallas.tpu as pltpu

F32 = jnp.float32
BF16 = jnp.bfloat16
U32 = jnp.uint32
HALO = 16
LANES = 128


def _butterfly(blocks):
    lane = jax.lax.broadcasted_iota(jnp.int32, blocks[0].shape, 1)
    for beta in (1, 2, 4):
        hi = (lane & (4 * beta)) != 0
        new = list(blocks)
        for j0 in range(8):
            if j0 & beta:
                continue
            j1 = j0 | beta
            new[j0] = jnp.where(hi, pltpu.roll(blocks[j1], 4 * beta, 1), blocks[j0])
            new[j1] = jnp.where(hi, blocks[j1], pltpu.roll(blocks[j0], LANES - 4 * beta, 1))
        blocks = new
    return blocks


def _opaque_zero(v):
    s = jnp.uint32(16)
    return jax.lax.shift_right_logical(jax.lax.shift_right_logical(v, s), s)


def _fzero(v):
    return pltpu.bitcast(_opaque_zero(pltpu.bitcast(v, U32)), F32)


def _silu(x):
    hx = 0.5 * x
    return hx * (1.0 + jnp.tanh(hx))


def _tree(op, xs):
    xs = list(xs)
    while len(xs) > 1:
        xs = [op(xs[i], xs[i + 1]) if i + 1 < len(xs) else xs[i] for i in range(0, len(xs), 2)]
    return xs[0]


def _pack(y):
    return pltpu.bitcast(y.astype(BF16), U32)


def build(A_x, A_wqkv, A_wo, B_x, B_w_gate, B_w_up, B_w_down, TM=256, FC=512,
          chunks=(128, 256, 256, 384, 384, 384, 256), chain=1, pchain=3, lng=32, lnchain=1, opaque=True, ser=1, serv=1, SR=16, split=None, ln1=None, bigat=5, ln1chain=4, nochk=True, pall=False, wpad=128, dpad=0, xnu=True, osplit=(768, 256), midk='pv', nextk='all', fastinv=True, postnorm=True, scopes=False):
    scope = jax.named_scope if scopes else (lambda name: contextlib.nullcontext())
    B, S, D = A_x.shape
    F = B_w_gate.shape[1]
    H = 32
    Dh = D // H
    W, dil = 8, 2
    scale = Dh ** -0.5
    NB = D // LANES
    NT = S // TM
    RC = 16
    TH = TM // 2
    NWC = len(chunks)
    assert sum(chunks) == 2 * D
    nsplit = NWC if split is None else split
    nln1 = NWC - 1 if ln1 is None else ln1
    chunk_off = [sum(chunks[:n]) for n in range(NWC)]
    x2 = A_x.reshape(S, D)

    def kernel(x_hbm, wqkv_hbm, wo_hbm, wg_hbm, wu_hbm, wd_hbm, o_hbm,
               x_buf, xn_buf, wqkv, wo, wg, wu, wd, kv_raw, q_buf, k_buf, v_buf, a_buf, o_buf, off_tab,
               x_sem, wc_sem, w_sem, o_sem):
        def tile_rows(t):
            return pl.ds(pl.multiple_of(t * TM, TM), TM)

        def half_rows(t):
            return pl.ds(pl.multiple_of(t * TH, TH), TH)

        def x_cp(t):
            return pltpu.make_async_copy(x_hbm.at[tile_rows(t), :], x_buf.at[tile_rows(t), :], x_sem.at[t])

        def o_cp(t, p):
            cols = pl.ds(sum(osplit[:p]), osplit[p])
            return pltpu.make_async_copy(o_buf.at[tile_rows(t), cols], o_hbm.at[tile_rows(t), cols],
                                         o_sem.at[t * len(osplit) + p])

        def wc_cp(n):
            cols = pl.ds(D + chunk_off[n], chunks[n])
            return pltpu.make_async_copy(wqkv_hbm.at[:, cols], wqkv.at[:, cols], wc_sem.at[n])

        big = [(wqkv_hbm.at[:, 0:D], wqkv.at[:, 0:D]), (wg_hbm, wg), (wu_hbm, wu), (wd_hbm, wd.at[:, 0:D]), (wo_hbm, wo.at[:, 0:D])]

        def w_cp(n):
            return pltpu.make_async_copy(big[n][0], big[n][1], w_sem.at[n])

        def layernorm(t, nchain=0):
            deps = []
            step = lng if nchain else TM
            for r in range(0, TM, step):
                rows = pl.ds(pl.multiple_of(t * TM + r, step), step)
                x = x_buf[rows, :].astype(F32)
                m = jnp.mean(x, axis=-1, keepdims=True)
                if nchain and len(deps) >= nchain:
                    m = m + pltpu.bitcast(_opaque_zero(deps[-nchain]), F32)
                xc = x - m
                var = jnp.mean(xc * xc, axis=-1, keepdims=True)
                xn = xc * jax.lax.rsqrt(var + 1e-5)
                if nchain:
                    deps.append(pltpu.bitcast(xn[:, D - 1:D], U32))
                if xnu:
                    xn_buf[pl.ds(pl.multiple_of(t * TH + r // 2, step // 2), step // 2), :] = _pack(xn)
                else:
                    xn_buf[rows, :] = xn.astype(BF16)

        def load_xn(t):
            return pltpu.bitcast(xn_buf[half_rows(t), :], BF16) if xnu else xn_buf[tile_rows(t), :]

        def phase_a0():
            for n in range(NWC):
                with scope(f"wcwait{n}"):
                    wc_cp(n).wait()
                if n == 0:
                    x_cp(1).start(priority=1)
                if n == 1:
                    for m in range(nsplit, NWC):
                        wc_cp(m).start(priority=1)
                if n == bigat:
                    for m in range(len(big)):
                        w_cp(m).start(priority=1)
                if n == NWC - 1:
                    for tt in range(2, NT):
                        x_cp(tt).start()
                if n == nln1:
                    with scope("x1wait"):
                        x_cp(1).wait()
                    layernorm(1, ln1chain)
                c0, cw = chunk_off[n], chunks[n]
                kv_raw[0:TH, c0:c0 + cw] = _pack(
                    jnp.dot(load_xn(0), wqkv[:, D + c0:D + c0 + cw], preferred_element_type=F32))

        def phase_a(t):
            kv_raw[half_rows(t), :] = _pack(
                jnp.dot(load_xn(t), wqkv[:, D:3 * D], preferred_element_type=F32))
            layernorm(jnp.minimum(t + 1, NT - 1), lnchain)

        def permute_kv(t):
            deps = []
            for r in range(0, TM, 16):
                for part, dst in ((0, k_buf), (1, v_buf)):
                    src_rows = pl.ds(pl.multiple_of(t * TH + r // 2, 8), 8)
                    blocks = [kv_raw[src_rows, part * D + LANES * j:part * D + LANES * (j + 1)] for j in range(NB)]
                    if len(deps) >= pchain:
                        zero = _opaque_zero(deps[-pchain])
                        blocks = [b | zero for b in blocks]
                    blocks = _butterfly(blocks)
                    deps.append(_tree(jnp.bitwise_or, blocks) if pall else blocks[NB - 1])
                    for j in range(NB):
                        dst[j, pl.ds(pl.multiple_of(t * TM + HALO + r, 8), 16), :] = (
                            pltpu.bitcast(blocks[j], BF16).astype(F32))
            dep = deps[-1]
            for d in deps[-pchain:-1]:
                dep = dep | d
            return dep

        lane = jax.lax.broadcasted_iota(jnp.int32, (SR, LANES), 1)
        odd = (lane & 1) == 1
        hi2 = (lane & 2) == 2
        rowi = jax.lax.broadcasted_iota(jnp.int32, (SR, LANES), 0)
        cexp = scale * math.log2(math.e)

        def attn_rows(t, row0, r0, qs, dep):
            base = row0 + (HALO + r0)
            logits = []
            raws = [dep] * ser
            for w in range(W):
                acc = qs[0] * k_buf[0, pl.ds(base - dil * w, SR), :]
                if raws[-ser] is not None:
                    acc = acc + _fzero(raws[-ser])
                for j in range(1, NB):
                    acc = acc + qs[j] * k_buf[j, pl.ds(base - dil * w, SR), :]
                raws.append(acc)
                acc = acc + jnp.where(odd, pltpu.roll(acc, 1, 1), pltpu.roll(acc, LANES - 1, 1))
                acc = acc + jnp.where(hi2, pltpu.roll(acc, 2, 1), pltpu.roll(acc, LANES - 2, 1))
                if w > 0 and r0 < dil * w:
                    pos = rowi + (t * TM + r0 - dil * w)
                    acc = jnp.where(pos >= 0, acc, -1e9 / scale)
                logits.append(acc)
            mx = _tree(jnp.maximum, logits)
            ps = [jnp.exp2((l - mx) * cexp) for l in logits]
            den = _tree(jnp.add, ps)
            if fastinv:
                r = pl.reciprocal(den, approx=True)
                inv = r * (2.0 - den * r)
            else:
                inv = 1.0 / den
            if not postnorm:
                ps = [p * inv for p in ps]
            raws = []
            outs = []
            for j in range(NB):
                o = ps[0] * v_buf[j, pl.ds(base, SR), :]
                if serv and j >= serv:
                    o = o + _fzero(raws[-serv])
                for w in range(1, W):
                    o = o + ps[w] * v_buf[j, pl.ds(base - dil * w, SR), :]
                raws.append(o)
                outs.append(o * inv if postnorm else o)
            mid = {"sm": inv, "pv": raws[-1], "qk": logits[-1]}[midk]
            return outs, mid

        def attn_chunk(t, row0, r0, dep):
            zero = _opaque_zero(dep)
            qb = _butterfly([q_buf[r0 // 2:(r0 + RC) // 2, LANES * j:LANES * (j + 1)] | zero for j in range(NB)])
            qs = [pltpu.bitcast(b, BF16).astype(F32) for b in qb]
            parts = []
            mid = None
            for h in range(0, RC, SR):
                o, mid = attn_rows(t, row0, r0 + h, [q[h:h + SR] for q in qs], mid)
                parts.append(o)
            ob = _butterfly([_pack(jnp.concatenate([p[j] for p in parts], axis=0)) for j in range(NB)])
            for j in range(NB):
                a_buf[r0 // 2:(r0 + RC) // 2, LANES * j:LANES * (j + 1)] = ob[j]
            return {"end": ob[NB - 1], "all": _tree(jnp.bitwise_or, ob), "mid": pltpu.bitcast(mid[0:8], U32)}[nextk]

        def phase_b(t):
            rows = tile_rows(t)
            xn = load_xn(t)
            q_buf[...] = _pack(jnp.dot(xn, wqkv[:, 0:D], preferred_element_type=F32))
            deps = [permute_kv(t)] * chain
            row0 = off_tab[t] if opaque else t * TM
            for r0 in range(0, TM, RC):
                deps.append(attn_chunk(t, row0, r0, deps[-chain]))
            acc = None
            for c in range(F // FC):
                g = jnp.dot(xn, wg[:, c * FC:(c + 1) * FC], preferred_element_type=F32)
                u = jnp.dot(xn, wu[:, c * FC:(c + 1) * FC], preferred_element_type=F32)
                h = (_silu(g) * u).astype(BF16)
                d = jnp.dot(h, wd[c * FC:(c + 1) * FC, 0:D], preferred_element_type=F32)
                acc = d if acc is None else acc + d
            a = pltpu.bitcast(a_buf[...], BF16)
            for p in range(len(osplit)):
                c0, c1 = sum(osplit[:p]), sum(osplit[:p + 1])
                s = jnp.dot(a, wo[:, c0:c1], preferred_element_type=F32)
                o_buf[rows, c0:c1] = (x_buf[rows, c0:c1].astype(F32) + s * _silu(acc[:, c0:c1])).astype(BF16)
                o_cp(t, p).start()

        x_cp(0).start()
        wc_cp(0).start(priority=1)
        for t in range(NT):
            off_tab[t] = t * TM
        k_buf[:, 0:HALO, :] = jnp.zeros((NB, HALO, LANES), F32)
        v_buf[:, 0:HALO, :] = jnp.zeros((NB, HALO, LANES), F32)
        with scope("x0wait"):
            x_cp(0).wait()
        for n in range(1, nsplit):
            wc_cp(n).start(priority=1)
        with scope("ln0"):
            layernorm(0)
        phase_a0()

        def a_body(t, c):
            @pl.when(t + 1 < NT)
            def _():
                x_cp(t + 1).wait()
            with scope("A"):
                phase_a(t)
            return c
        jax.lax.fori_loop(1, NT, a_body, 0)

        with scope("bigwait"):
            for n in range(len(big)):
                w_cp(n).wait()

        def b_body(t, c):
            with scope("B"):
                phase_b(t)
            return c
        jax.lax.fori_loop(0, NT, b_body, 0)
        with scope("owait"):
            for t in range(NT):
                for p in range(len(osplit)):
                    o_cp(t, p).wait()

    anyspec = pl.BlockSpec(memory_space=pl.ANY)
    out = pl.pallas_call(
        kernel,
        in_specs=[anyspec] * 6,
        out_specs=anyspec,
        out_shape=jax.ShapeDtypeStruct((S, D), A_x.dtype),
        scratch_shapes=[
            pltpu.VMEM((S, D), BF16), pltpu.VMEM((S // 2, D), U32) if xnu else pltpu.VMEM((S, D), BF16),
            pltpu.VMEM((D, 3 * D + wpad), BF16), pltpu.VMEM((D, D + dpad), BF16),
            pltpu.VMEM((D, F), BF16), pltpu.VMEM((D, F), BF16), pltpu.VMEM((F, D + dpad), BF16),
            pltpu.VMEM((S // 2, 2 * D), U32), pltpu.VMEM((TH, D), U32),
            pltpu.VMEM((NB, S + HALO, LANES), F32), pltpu.VMEM((NB, S + HALO, LANES), F32),
            pltpu.VMEM((TH, D), U32), pltpu.VMEM((S, D), BF16), pltpu.SMEM((NT,), jnp.int32),
            pltpu.SemaphoreType.DMA((NT,)), pltpu.SemaphoreType.DMA((NWC,)),
            pltpu.SemaphoreType.DMA((5,)), pltpu.SemaphoreType.DMA((NT * len(osplit),)),
        ],
        compiler_params=pltpu.CompilerParams(vmem_limit_bytes=110 * 1024 * 1024, disable_bounds_checks=nochk,
                                             disable_semaphore_checks=nochk),
    )(x2, A_wqkv, A_wo, B_w_gate, B_w_up, B_w_down)
    return out.reshape(B, S, D)


@jax.jit
def pallas_recurrent_scan__sliding_local_dilated__swiglu_ffn__prompt_kernel(A_x, A_wqkv, A_wo, B_x, B_w_gate, B_w_up, B_w_down):
    return build(A_x, A_wqkv, A_wo, B_x, B_w_gate, B_w_up, B_w_down)
```

```python
import contextlib
import math
import jax
import jax.numpy as jnp
import jax.experimental.pallas as pl
import jax.experimental.pallas.tpu as pltpu

F32 = jnp.float32
BF16 = jnp.bfloat16
U32 = jnp.uint32
HALO = 16
LANES = 128
SLOT = (4, 0, 2, 1, 3, 5, 6)


def _butterfly(blocks):
    lane = jax.lax.broadcasted_iota(jnp.int32, blocks[0].shape, 1)
    for beta in (1, 2, 4):
        hi = (lane & (4 * beta)) != 0
        new = list(blocks)
        for j0 in range(8):
            if j0 & beta:
                continue
            j1 = j0 | beta
            new[j0] = jnp.where(hi, pltpu.roll(blocks[j1], 4 * beta, 1), blocks[j0])
            new[j1] = jnp.where(hi, blocks[j1], pltpu.roll(blocks[j0], LANES - 4 * beta, 1))
        blocks = new
    return blocks


def _opaque_zero(v):
    s = jnp.uint32(16)
    return jax.lax.shift_right_logical(jax.lax.shift_right_logical(v, s), s)


def _fzero(v):
    return pltpu.bitcast(_opaque_zero(pltpu.bitcast(v, U32)), F32)


def _silu(x):
    hx = 0.5 * x
    return hx * (1.0 + jnp.tanh(hx))


def _tree(op, xs):
    xs = list(xs)
    while len(xs) > 1:
        xs = [op(xs[i], xs[i + 1]) if i + 1 < len(xs) else xs[i] for i in range(0, len(xs), 2)]
    return xs[0]


def _lhs_combos(a11, a12, a21, a22):
    return [a11 + a22, a21 + a22, a11, a22, a11 + a12, a21 - a11, a12 - a22]


def _combine(m):
    return m[0] + m[3] - m[4] + m[6], m[2] + m[4], m[1] + m[3], m[0] - m[1] + m[2] + m[5]


def _pack(y):
    return pltpu.bitcast(y.astype(BF16), U32)


def _dot(a, b):
    return jnp.dot(a, b, preferred_element_type=F32)


def build(A_x, A_wqkv, A_wo, B_x, B_w_gate, B_w_up, B_w_down,
          subs=(128, 128, 256, 256, 256, 256, 128, 128), x1at=6, ln1=6, ln1chain=2, pchain=3, lnchain=1,
          PR=8, wchain=2, wroll=True, p0chain=2, scopes=False):
    scope = jax.named_scope if scopes else (lambda name: contextlib.nullcontext())
    B, S, D = A_x.shape
    F = B_w_gate.shape[1]
    H = 32
    Dh = D // H
    W, dil = 8, 2
    scale = Dh ** -0.5
    NB = D // LANES
    TM = 256
    NT = S // TM
    RC = 16
    TH = TM // 2
    TQ = TM // 4
    KH = D // 2
    FH = F // 2
    NH = 3 * D // 2
    CW = KH // 2
    NC = FH // CW
    UR = 256
    NU = 3 * NC + 2
    UPS = 4
    NS = NT - 2
    assert NS * UPS >= NU and sum(subs) == NH
    NSUB = len(subs)
    sub_off = [sum(subs[:n]) for n in range(NSUB)]
    assert all(o // KH == (o + s - 1) // KH for o, s in zip(sub_off, subs))

    def kernel(x_hbm, wqkv_hbm, wo_hbm, wg_hbm, wu_hbm, wd_hbm, o_hbm,
               x_buf, xn0, xs_buf, wa, wb, qkv_raw, k_buf, v_buf, a_buf, o_buf, off_tab,
               x_sem, wa_sem, wb_sem, o_sem):
        def tile_rows(t):
            return pl.ds(pl.multiple_of(t * TM, TM), TM)

        def x_cp(t):
            return pltpu.make_async_copy(x_hbm.at[tile_rows(t), :], x_buf.at[tile_rows(t), :], x_sem.at[t])

        def o_cp(t):
            return pltpu.make_async_copy(o_buf.at[tile_rows(t), :], o_hbm.at[tile_rows(t), :], o_sem.at[t])

        def sub_pos(n):
            u, c = divmod(sub_off[n], KH)
            return pl.ds(u * KH, KH), pl.ds(c, subs[n])

        def wa_cps(n):
            rows, cols = sub_pos(n)
            return [pltpu.make_async_copy(wqkv_hbm.at[:, :, pl.ds(j * NH + sub_off[n], subs[n])],
                                          wa.at[pl.ds(2 * j, 2), rows, cols], wa_sem.at[n]) for j in range(2)]

        def wb_cps(s):
            cps = []
            for u in range(s * UPS, min((s + 1) * UPS, NU)):
                rows = pl.ds(u * UR, UR)
                c, part = divmod(u, 3)
                for j in range(2):
                    dst = wb.at[pl.ds(2 * j, 2), rows, :]
                    if c == NC:
                        srcs = [(wo_hbm.at[:, pl.ds(part * UR, UR), pl.ds(j * KH, KH)], dst)]
                    elif part == 2:
                        srcs = [(wd_hbm.at[:, pl.ds(c * CW, CW), pl.ds(j * KH, KH)], dst)]
                    else:
                        srcs = [(w.at[:, pl.ds(part * UR, UR), pl.ds(j * FH + c * CW, CW)],
                                 wb.at[pl.ds(2 * j, 2), rows, pl.ds(n * CW, CW)])
                                for n, w in enumerate((wg_hbm, wu_hbm))]
                    cps += [pltpu.make_async_copy(a, b, wb_sem.at[s]) for a, b in srcs]
            return cps

        def layernorm(t, nchain, keep_plain=False):
            deps = []
            g = 16
            for r in range(0, TH, g):
                x = jnp.concatenate(
                    [x_buf[pl.ds(pl.multiple_of(t * TM + h * TH + r, g), g), :].astype(F32) for h in range(2)], axis=0)
                m = jnp.mean(x, axis=-1, keepdims=True)
                if nchain and len(deps) >= nchain:
                    m = m + pltpu.bitcast(_opaque_zero(deps[-nchain]), F32)
                xc = x - m
                var = jnp.mean(xc * xc, axis=-1, keepdims=True)
                xn = xc * jax.lax.rsqrt(var + 1e-5)
                deps.append(pltpu.bitcast(xn[:, D - 1:D], U32))
                if keep_plain:
                    xp = _pack(xn)
                    for h in range(2):
                        xn0[h * TQ + r // 2:h * TQ + (r + g) // 2, :] = xp[h * g // 2:(h + 1) * g // 2]
                cp = _pack(jnp.concatenate(_lhs_combos(xn[:g, :KH], xn[:g, KH:], xn[g:, :KH], xn[g:, KH:]), axis=0))
                for n in range(7):
                    xs_buf[n, pl.ds(pl.multiple_of(t * TQ + r // 2, g // 2), g // 2), :] = cp[n * g // 2:(n + 1) * g // 2]

        def prep(w, row0, nrows, cols, nchain, roll, PR=PR):
            deps = []
            for r in range(0, nrows, PR):
                rows = pl.ds(row0 + r, PR) if isinstance(row0, int) else pl.ds(pl.multiple_of(row0 + r, PR), PR)
                b11, b21, b12, b22 = [w[s, rows, cols].astype(F32) for s in range(4)]
                if nchain and len(deps) >= nchain:
                    z = _fzero(deps[-nchain])
                    if roll:
                        z = pltpu.roll(z, 1, 1)
                    z = jnp.concatenate([z] * (b11.shape[1] // LANES), axis=1)
                    b11 = b11 + z
                    b22 = b22 + z
                last = b21 + b22
                deps.append(last[:, :LANES])
                w[4, rows, cols] = (b11 + b22).astype(BF16)
                w[2, rows, cols] = (b12 - b22).astype(BF16)
                w[1, rows, cols] = (b21 - b11).astype(BF16)
                w[5, rows, cols] = (b11 + b12).astype(BF16)
                w[6, rows, cols] = last.astype(BF16)

        def load_lhs(t):
            rows = pl.ds(pl.multiple_of(t * TQ, TQ), TQ)
            return [pltpu.bitcast(xs_buf[n, rows, :], BF16) for n in range(7)]

        def phase_a0():
            for n in range(NSUB + 1):
                if n < NSUB:
                    with scope(f"wawait{n}"):
                        for cp in wa_cps(n):
                            cp.wait()
                if n == 0:
                    x_cp(1).start()
                if n == 1:
                    for m in range(x1at, NSUB):
                        for cp in wa_cps(m):
                            cp.start()
                if n == NSUB - 2:
                    for cp in wb_cps(0):
                        cp.start()
                if n == NSUB - 3:
                    x_cp(2).start()
                if n == ln1:
                    with scope("x1wait"):
                        x_cp(1).wait()
                    layernorm(1, ln1chain)
                if n > 0:
                    rows, cols = sub_pos(n - 1)
                    prep(wa, rows.start, KH, cols, p0chain if n < NSUB else 0, True, PR=16 if (n < NSUB and subs[n] >= 256) else 32)
                if n < NSUB:
                    rows, cols = sub_pos(n)
                    xn = pltpu.bitcast(xn0[...], BF16)
                    for j in range(2):
                        wj = jnp.concatenate([wa[2 * j, rows, cols], wa[2 * j + 1, rows, cols]], axis=0)
                        c0 = j * NH + sub_off[n]
                        qkv_raw[0:TH, c0:c0 + subs[n]] = _pack(_dot(xn, wj))

        def phase_a(t):
            lhs = load_lhs(t)
            for u in range(NH // KH):
                quads = _combine([_dot(lhs[i], wa[SLOT[i], u * KH:(u + 1) * KH, :]) for i in range(7)])
                for n, y in enumerate(quads):
                    i, j = divmod(n, 2)
                    qkv_raw[pl.ds(pl.multiple_of(t * TH + i * TQ, TQ), TQ), j * NH + u * KH:j * NH + (u + 1) * KH] = _pack(y)
            layernorm(jnp.minimum(t + 1, NT - 1), lnchain)
            s = jnp.where(t >= 2, t - 2, NS - 1)
            prep(wb, s * (UPS * UR), UPS * UR, slice(None), wchain, wroll)

        def permute_kv(t):
            deps = []
            for r in range(0, TM, 16):
                for part, dst in ((1, k_buf), (2, v_buf)):
                    src_rows = pl.ds(pl.multiple_of(t * TH + r // 2, 8), 8)
                    blocks = [qkv_raw[src_rows, part * D + LANES * j:part * D + LANES * (j + 1)] for j in range(NB)]
                    if len(deps) >= pchain:
                        zero = _opaque_zero(deps[-pchain])
                        blocks = [b | zero for b in blocks]
                    blocks = _butterfly(blocks)
                    deps.append(blocks[NB - 1])
                    for j in range(NB):
                        dst[j, pl.ds(pl.multiple_of(t * TM + HALO + r, 8), 16), :] = (
                            pltpu.bitcast(blocks[j], BF16).astype(F32))
            return _tree(jnp.bitwise_or, deps[-pchain:])

        lane = jax.lax.broadcasted_iota(jnp.int32, (RC, LANES), 1)
        odd = (lane & 1) == 1
        hi2 = (lane & 2) == 2
        rowi = jax.lax.broadcasted_iota(jnp.int32, (RC, LANES), 0)
        cexp = scale * math.log2(math.e)

        def attn_chunk(t, row0, r0, dep):
            zero = _opaque_zero(dep)
            qrows = pl.ds(pl.multiple_of(t * TH + r0 // 2, 8), RC // 2)
            qb = _butterfly([qkv_raw[qrows, LANES * j:LANES * (j + 1)] | zero for j in range(NB)])
            qs = [pltpu.bitcast(b, BF16).astype(F32) for b in qb]
            base = row0 + (HALO + r0)
            logits = []
            prev = None
            for w in range(W):
                acc = qs[0] * k_buf[0, pl.ds(base - dil * w, RC), :]
                if prev is not None:
                    acc = acc + _fzero(prev)
                for j in range(1, NB):
                    acc = acc + qs[j] * k_buf[j, pl.ds(base - dil * w, RC), :]
                prev = acc
                acc = acc + jnp.where(odd, pltpu.roll(acc, 1, 1), pltpu.roll(acc, LANES - 1, 1))
                acc = acc + jnp.where(hi2, pltpu.roll(acc, 2, 1), pltpu.roll(acc, LANES - 2, 1))
                if w > 0 and r0 < dil * w:
                    pos = rowi + (t * TM + r0 - dil * w)
                    acc = jnp.where(pos >= 0, acc, -1e9 / scale)
                logits.append(acc)
            mx = _tree(jnp.maximum, logits)
            ps = [jnp.exp2((l - mx) * cexp) for l in logits]
            den = _tree(jnp.add, ps)
            r = pl.reciprocal(den, approx=True)
            inv = r * (2.0 - den * r)
            outs = []
            prev = None
            for j in range(NB):
                o = ps[0] * v_buf[j, pl.ds(base, RC), :]
                if prev is not None:
                    o = o + _fzero(prev)
                for w in range(1, W):
                    o = o + ps[w] * v_buf[j, pl.ds(base - dil * w, RC), :]
                prev = o
                outs.append(_pack(o * inv))
            ob = _butterfly(outs)
            for j in range(NB):
                a_buf[r0 // 2:(r0 + RC) // 2, LANES * j:LANES * (j + 1)] = ob[j]
            return _tree(jnp.bitwise_or, ob)

        def phase_b(t):
            dep = permute_kv(t)
            row0 = off_tab[t]
            for r0 in range(0, TM, RC):
                dep = attn_chunk(t, row0, r0, dep)
            lhs = load_lhs(t)
            accs = [None] * 7
            for c in range(NC):
                u0 = 3 * c * UR
                gu = _combine([_dot(lhs[i], wb[SLOT[i], u0:u0 + KH, :]) for i in range(7)])
                hl = _lhs_combos(*[_silu(z[:, :CW]) * z[:, CW:] for z in gu])
                for i in range(7):
                    d = _dot(hl[i].astype(BF16), wb[SLOT[i], u0 + KH:u0 + KH + CW, :])
                    accs[i] = d if accs[i] is None else accs[i] + d
            ys = _combine(accs)
            a = pltpu.bitcast(a_buf[...], BF16).astype(F32)
            al = _lhs_combos(a[:TH, :KH], a[:TH, KH:], a[TH:, :KH], a[TH:, KH:])
            u0 = 3 * NC * UR
            ss = _combine([_dot(al[i].astype(BF16), wb[SLOT[i], u0:u0 + KH, :]) for i in range(7)])
            for n in range(4):
                i, j = divmod(n, 2)
                rows = pl.ds(pl.multiple_of(t * TM + i * TH, TH), TH)
                cols = slice(j * KH, (j + 1) * KH)
                o_buf[rows, cols] = (x_buf[rows, cols].astype(F32) + ss[n] * _silu(ys[n])).astype(BF16)
            o_cp(t).start()

        x_cp(0).start()
        for cp in wa_cps(0):
            cp.start()
        for t in range(NT):
            off_tab[t] = t * TM
        k_buf[:, 0:HALO, :] = jnp.zeros((NB, HALO, LANES), F32)
        v_buf[:, 0:HALO, :] = jnp.zeros((NB, HALO, LANES), F32)
        with scope("x0wait"):
            x_cp(0).wait()
        for n in range(1, x1at):
            for cp in wa_cps(n):
                cp.start()
        with scope("ln0"):
            layernorm(0, 0, keep_plain=True)
        phase_a0()

        def a_body(t, c):
            with scope("Await"):
                @pl.when(t + 1 < NT)
                def _():
                    x_cp(t + 1).wait()

                @pl.when(t + 2 < NT)
                def _():
                    x_cp(t + 2).start()
                for s in range(NS):
                    @pl.when(t == s + 2)
                    def _():
                        for cp in wb_cps(s):
                            cp.wait()
                for s in range(1, NS):
                    @pl.when(t == s)
                    def _():
                        for cp in wb_cps(s):
                            cp.start()
            with scope("A"):
                phase_a(t)
            return c
        jax.lax.fori_loop(1, NT, a_body, 0)

        def b_body(t, c):
            with scope("B"):
                phase_b(t)
            return c
        jax.lax.fori_loop(0, NT, b_body, 0)
        with scope("owait"):
            for t in range(NT):
                o_cp(t).wait()

    anyspec = pl.BlockSpec(memory_space=pl.ANY)
    out = pl.pallas_call(
        kernel,
        in_specs=[anyspec] * 6,
        out_specs=anyspec,
        out_shape=jax.ShapeDtypeStruct((S, D), A_x.dtype),
        scratch_shapes=[
            pltpu.VMEM((S, D), BF16), pltpu.VMEM((TH, D), U32), pltpu.VMEM((7, S // 4, KH), U32),
            pltpu.VMEM((7, NH, KH), BF16), pltpu.VMEM((7, NS * UPS * UR, KH), BF16),
            pltpu.VMEM((S // 2, 3 * D), U32),
            pltpu.VMEM((NB, S + HALO, LANES), F32), pltpu.VMEM((NB, S + HALO, LANES), F32),
            pltpu.VMEM((TH, D), U32), pltpu.VMEM((S, D), BF16), pltpu.SMEM((NT,), jnp.int32),
            pltpu.SemaphoreType.DMA((NT,)), pltpu.SemaphoreType.DMA((NSUB,)),
            pltpu.SemaphoreType.DMA((NS,)), pltpu.SemaphoreType.DMA((NT,)),
        ],
        compiler_params=pltpu.CompilerParams(vmem_limit_bytes=124 * 1024 * 1024, disable_bounds_checks=True,
                                             disable_semaphore_checks=True),
    )(A_x.reshape(S, D), A_wqkv.reshape(2, KH, 3 * D), A_wo.reshape(2, KH, D),
      B_w_gate.reshape(2, KH, F), B_w_up.reshape(2, KH, F), B_w_down.reshape(2, FH, D))
    return out.reshape(B, S, D)


@jax.jit
def pallas_recurrent_scan__sliding_local_dilated__swiglu_ffn__prompt_kernel(A_x, A_wqkv, A_wo, B_x, B_w_gate, B_w_up, B_w_down):
    return build(A_x, A_wqkv, A_wo, B_x, B_w_gate, B_w_up, B_w_down)
```

```python
import contextlib
import math
import jax
import jax.numpy as jnp
import jax.experimental.pallas as pl
import jax.experimental.pallas.tpu as pltpu

F32 = jnp.float32
BF16 = jnp.bfloat16
U32 = jnp.uint32
HALO = 16
LANES = 128
QORDER = (2, 1, 3, 0)


def _butterfly(blocks):
    lane = jax.lax.broadcasted_iota(jnp.int32, blocks[0].shape, 1)
    for beta in (1, 2, 4):
        hi = (lane & (4 * beta)) != 0
        new = list(blocks)
        for j0 in range(8):
            if j0 & beta:
                continue
            j1 = j0 | beta
            new[j0] = jnp.where(hi, pltpu.roll(blocks[j1], 4 * beta, 1), blocks[j0])
            new[j1] = jnp.where(hi, blocks[j1], pltpu.roll(blocks[j0], LANES - 4 * beta, 1))
        blocks = new
    return blocks


def _opaque_zero(v):
    s = jnp.uint32(16)
    return jax.lax.shift_right_logical(jax.lax.shift_right_logical(v, s), s)


def _fzero(v):
    return pltpu.bitcast(_opaque_zero(pltpu.bitcast(v, U32)), F32)


def _silu(x):
    hx = 0.5 * x
    return hx * (1.0 + jnp.tanh(hx))


def _tree(op, xs):
    xs = list(xs)
    while len(xs) > 1:
        xs = [op(xs[i], xs[i + 1]) if i + 1 < len(xs) else xs[i] for i in range(0, len(xs), 2)]
    return xs[0]


def _lhs_combos(a11, a12, a21, a22):
    return [a11 + a22, a21 + a22, a11, a22, a11 + a12, a21 - a11, a12 - a22]


def _combine(m):
    return m[0] + m[3] - m[4] + m[6], m[2] + m[4], m[1] + m[3], m[0] - m[1] + m[2] + m[5]


def _pack(y):
    return pltpu.bitcast(y.astype(BF16), U32)


def _dot(a, b):
    return jnp.dot(a, b, preferred_element_type=F32)


def build(A_x, A_wqkv, A_wo, B_x, B_w_gate, B_w_up, B_w_down,
          subs=(128, 128, 256, 256, 256, 256, 128, 128), x1at=6, ln1=(6, 7), ln1chain=2, pchain=3, lnchain=1,
          PR=16, CG=256, lnfirst=False, mchain=0, lean=0, LCG=256, lndep2=True, wchain=2, p0chain=2, scopes=False):
    scope = jax.named_scope if scopes else (lambda name: contextlib.nullcontext())
    B, S, D = A_x.shape
    F = B_w_gate.shape[1]
    H = 32
    Dh = D // H
    W, dil = 8, 2
    scale = Dh ** -0.5
    NB = D // LANES
    TM = 256
    NT = S // TM
    RC = 16
    TH = TM // 2
    TQ = TM // 4
    KH = D // 2
    FH = F // 2
    NH = 3 * D // 2
    CW = KH // 2
    NC = FH // CW
    UR = 256
    NU = 3 * NC + 2
    UPS = 4
    NS = NT - 2
    SR = UPS * UR
    RING = 3
    assert NS * UPS >= NU and sum(subs) == NH
    NSUB = len(subs)
    sub_off = [sum(subs[:n]) for n in range(NSUB)]
    assert all(o // KH == (o + s - 1) // KH for o, s in zip(sub_off, subs))

    def kernel(x_hbm, wqkv_hbm, wo_hbm, wg_hbm, wu_hbm, wd_hbm, o_hbm,
               x_buf, xn0, xs_buf, wa, wa_p, wb, wb_p, qkv_raw, k_buf, v_buf, a_buf, o_buf, off_tab,
               x_sem, wa_sem, wb_sem, o_sem):
        def tile_rows(t):
            return pl.ds(pl.multiple_of(t * TM, TM), TM)

        def x_cp(t):
            return pltpu.make_async_copy(x_hbm.at[tile_rows(t), :], x_buf.at[tile_rows(t), :], x_sem.at[t])

        def quad_pos(t, n):
            i, j = divmod(n, 2)
            return pl.ds(pl.multiple_of(t * TM + i * TH, TH), TH), pl.ds(j * KH, KH)

        def o_cp(t, n):
            rows, cols = quad_pos(t, n)
            return pltpu.make_async_copy(o_buf.at[rows, cols], o_hbm.at[rows, cols], o_sem.at[4 * t + n])

        def sub_pos(n):
            u, c = divmod(sub_off[n], KH)
            return pl.ds(u * KH, KH), pl.ds(c, subs[n])

        def wa_cps(n):
            rows, cols = sub_pos(n)
            return [pltpu.make_async_copy(wqkv_hbm.at[:, :, pl.ds(j * NH + sub_off[n], subs[n])],
                                          wa.at[pl.ds(2 * j, 2), rows, cols], wa_sem.at[n]) for j in range(2)]

        def wb_cps(s):
            cps = []
            for u in range(s * UPS, min((s + 1) * UPS, NU)):
                rows = pl.ds((s % RING) * SR + (u - s * UPS) * UR, UR)
                c, part = divmod(u, 3)
                for j in range(2):
                    dst = wb.at[pl.ds(2 * j, 2), rows, :]
                    if c == NC:
                        srcs = [(wo_hbm.at[:, pl.ds(part * UR, UR), pl.ds(j * KH, KH)], dst)]
                    elif part == 2:
                        srcs = [(wd_hbm.at[:, pl.ds(c * CW, CW), pl.ds(j * KH, KH)], dst)]
                    else:
                        srcs = [(w.at[:, pl.ds(part * UR, UR), pl.ds(j * FH + c * CW, CW)],
                                 wb.at[pl.ds(2 * j, 2), rows, pl.ds(n * CW, CW)])
                                for n, w in enumerate((wg_hbm, wu_hbm))]
                    cps += [pltpu.make_async_copy(a, b, wb_sem.at[s]) for a, b in srcs]
            return cps

        def layernorm(t, nchain, keep_plain=False, dep0=None, r_lo=0, r_hi=TH):
            deps = [] if dep0 is None else [dep0] * nchain
            g = 16
            for r in range(r_lo, r_hi, g):
                x = jnp.concatenate(
                    [x_buf[pl.ds(pl.multiple_of(t * TM + h * TH + r, g), g), :].astype(F32) for h in range(2)], axis=0)
                m = jnp.mean(x, axis=-1, keepdims=True)
                if nchain and len(deps) >= nchain:
                    m = m + pltpu.bitcast(_opaque_zero(deps[-nchain]), F32)
                xc = x - m
                var = jnp.mean(xc * xc, axis=-1, keepdims=True)
                xn = xc * jax.lax.rsqrt(var + 1e-5)
                deps.append(pltpu.bitcast(xn[:, D - 1:D], U32))
                if keep_plain:
                    for h in range(2):
                        xn0[h * TQ + r // 2:h * TQ + (r + g) // 2, :] = _pack(xn[h * g:(h + 1) * g])
                combos = _lhs_combos(xn[:g, :KH], xn[:g, KH:], xn[g:, :KH], xn[g:, KH:])
                for n in range(7):
                    xs_buf[pl.ds(pl.multiple_of(n * (S // 4) + t * TQ + r // 2, g // 2), g // 2), :] = _pack(combos[n])
            return pltpu.bitcast(combos[6][0:8, 0:LANES], U32)

        def layernorm_lean(t, nchain):
            g = 16
            zoff = off_tab[0]
            deps = []
            for r in range(0, TH, g):
                stats = []
                for h in range(2):
                    for q in range(0, g, 8):
                        x = x_buf[pl.ds(pl.multiple_of(t * TM + h * TH + r + q, 8), 8), :].astype(F32)
                        m = jnp.mean(x, axis=-1, keepdims=True)
                        if len(deps) >= nchain:
                            m = m + _fzero(deps[-nchain])[:, 0:1]
                        xc = x - m
                        var = jnp.mean(xc * xc, axis=-1, keepdims=True)
                        rs = jax.lax.rsqrt(var + 1e-5)
                        stats.append((m, rs))
                        deps.append(jnp.broadcast_to(rs, (8, LANES)))
                ms = [jnp.concatenate([stats[2 * h][0], stats[2 * h + 1][0]], axis=0) for h in range(2)]
                rss = [jnp.concatenate([stats[2 * h][1], stats[2 * h + 1][1]], axis=0) for h in range(2)]
                for c in range(0, KH, LCG):
                    quad = []
                    for h in range(2):
                        rows = pl.ds(pl.multiple_of(zoff + (t * TM + h * TH + r), g), g)
                        for j in range(2):
                            quad.append((x_buf[rows, j * KH + c:j * KH + c + LCG].astype(F32) - ms[h]) * rss[h])
                    combos = _lhs_combos(*quad)
                    for n in range(7):
                        xs_buf[pl.ds(pl.multiple_of(n * (S // 4) + t * TQ + r // 2, g // 2), g // 2), c:c + LCG] = (
                            _pack(combos[n]))
                if lndep2:
                    deps.append(combos[6][0:8, 0:LANES])

        def prep(w, row0, nrows, c0, ncols, dst, dst_row0, nchain, dep0=None):
            deps = [] if dep0 is None else [dep0] * nchain
            plane = dst.shape[0] // 7
            half0 = dst_row0 // 2
            cg = min(CG, ncols)
            for r in range(0, nrows, PR):
                rows = pl.ds(pl.multiple_of(row0 + r, PR), PR)
                for c in range(c0, c0 + ncols, cg):
                    cols = pl.ds(c, cg)
                    b11, b21, b12, b22 = [w[s, rows, cols].astype(F32) for s in range(4)]
                    if nchain and len(deps) >= nchain:
                        z = pltpu.roll(_fzero(deps[-nchain]), 1, 1)
                        z = jnp.concatenate([z] * (cg // LANES), axis=1)
                        b11 = b11 + z
                        b22 = b22 + z
                    outs = [b11 + b22, b11, b12 - b22, b21 - b11, b22, b11 + b12, b21 + b22]
                    deps.append(outs[6][:, :LANES])
                    for i in range(7):
                        dst[pl.ds(pl.multiple_of(half0 + (i * plane + r // 2), PR // 2), PR // 2), cols] = _pack(outs[i])
            return deps[-1]

        def rhs(dst, i, row0, nrows):
            plane = dst.shape[0] // 7
            return pltpu.bitcast(dst[i * plane + row0 // 2:i * plane + (row0 + nrows) // 2, :], BF16)

        def load_lhs(t):
            return [pltpu.bitcast(xs_buf[pl.ds(pl.multiple_of(n * (S // 4) + t * TQ, TQ), TQ), :], BF16)
                    for n in range(7)]

        def phase_a0():
            for n in range(NSUB + 1):
                if n < NSUB:
                    with scope(f"wawait{n}"):
                        for cp in wa_cps(n):
                            cp.wait()
                if n == ln1[0]:
                    with scope("x1wait"):
                        x_cp(1).wait()
                if n == 0:
                    x_cp(1).start()
                if n == 1:
                    for m in range(x1at, NSUB):
                        for cp in wa_cps(m):
                            cp.start()
                if n == NSUB - 3:
                    x_cp(2).start()
                if n == NSUB - 2:
                    for cp in wb_cps(0):
                        cp.start()
                if n in ln1:
                    k = ln1.index(n)
                    layernorm(1, ln1chain, r_lo=k * TH // len(ln1), r_hi=(k + 1) * TH // len(ln1))
                if n > 0:
                    rows, cols = sub_pos(n - 1)
                    prep(wa, rows.start, KH, cols.start, cols.size, wa_p, rows.start, 0 if n == NSUB else (p0chain if subs[n] >= 256 else 2 * p0chain))
                if n < NSUB:
                    rows, cols = sub_pos(n)
                    xn = pltpu.bitcast(xn0[...], BF16)
                    for j in range(2):
                        wj = jnp.concatenate([wa[2 * j, rows, cols], wa[2 * j + 1, rows, cols]], axis=0)
                        c0 = j * NH + sub_off[n]
                        qkv_raw[0:TH, c0:c0 + subs[n]] = _pack(_dot(xn, wj))

        def tie(lhs_u32, dep):
            z = _opaque_zero(pltpu.bitcast(dep, U32))
            top = jnp.concatenate([lhs_u32[:8, :LANES] | z, lhs_u32[:8, LANES:]], axis=1)
            return jnp.concatenate([top, lhs_u32[8:]], axis=0)

        def phase_a(t):
            lhs = load_lhs(t)
            hist = []
            for u in range(NH // KH):
                ms = []
                for i in range(7):
                    l = lhs[i]
                    if mchain and len(hist) >= mchain:
                        l = pltpu.bitcast(tie(pltpu.bitcast(l, U32), hist[-mchain]), BF16)
                    ms.append(_dot(l, rhs(wa_p, i, u * KH, KH)))
                    hist.append(ms[-1][TH - 8:, KH - LANES:])
                quads = _combine(ms)
                for n in QORDER:
                    i, j = divmod(n, 2)
                    qkv_raw[pl.ds(pl.multiple_of(t * TH + i * TQ, TQ), TQ), j * NH + u * KH:j * NH + (u + 1) * KH] = (
                        _pack(quads[n]))
            s = jnp.where(t >= 2, t - 2, NS - 1)
            d = None
            if lean:
                layernorm_lean(jnp.minimum(t + 1, NT - 1), lean)
            else:
                d = pltpu.bitcast(layernorm(jnp.minimum(t + 1, NT - 1), lnchain), F32)
                d = jnp.concatenate([d] * (PR // 8), axis=0)
            prep(wb, ((t + 1) % RING) * SR, SR, 0, KH, wb_p, s * SR, wchain, dep0=d if lnfirst else None)

        def permute_kv(t):
            deps = []
            for r in range(-HALO, TM, 16):
                src0 = jnp.maximum(t * TH + r // 2, 0) if r < 0 else t * TH + r // 2
                for part, dst in ((1, k_buf), (2, v_buf)):
                    src_rows = pl.ds(pl.multiple_of(src0, 8), 8)
                    blocks = [qkv_raw[src_rows, part * D + LANES * j:part * D + LANES * (j + 1)] for j in range(NB)]
                    if len(deps) >= pchain:
                        zero = _opaque_zero(deps[-pchain])
                        blocks = [b | zero for b in blocks]
                    blocks = _butterfly(blocks)
                    deps.append(blocks[NB - 1])
                    for j in range(NB):
                        dst[j, HALO + r:HALO + r + 16, :] = pltpu.bitcast(blocks[j], BF16).astype(F32)
            return _tree(jnp.bitwise_or, deps[-pchain:])

        lane = jax.lax.broadcasted_iota(jnp.int32, (RC, LANES), 1)
        odd = (lane & 1) == 1
        hi2 = (lane & 2) == 2
        rowi = jax.lax.broadcasted_iota(jnp.int32, (RC, LANES), 0)
        cexp = scale * math.log2(math.e)

        def attn_chunk(t, row0, r0, dep):
            zero = _opaque_zero(dep)
            qrows = pl.ds(pl.multiple_of(t * TH + r0 // 2, 8), RC // 2)
            qb = _butterfly([qkv_raw[qrows, LANES * j:LANES * (j + 1)] | zero for j in range(NB)])
            qs = [pltpu.bitcast(b, BF16).astype(F32) for b in qb]
            base = row0 + (HALO + r0)
            logits = []
            prev = None
            for w in range(W):
                acc = qs[0] * k_buf[0, pl.ds(base - dil * w, RC), :]
                if prev is not None:
                    acc = acc + _fzero(prev)
                for j in range(1, NB):
                    acc = acc + qs[j] * k_buf[j, pl.ds(base - dil * w, RC), :]
                prev = acc
                acc = acc + jnp.where(odd, pltpu.roll(acc, 1, 1), pltpu.roll(acc, LANES - 1, 1))
                acc = acc + jnp.where(hi2, pltpu.roll(acc, 2, 1), pltpu.roll(acc, LANES - 2, 1))
                if w > 0 and r0 < dil * w:
                    pos = rowi + (t * TM + r0 - dil * w)
                    acc = jnp.where(pos >= 0, acc, -1e9 / scale)
                logits.append(acc)
            mx = _tree(jnp.maximum, logits)
            ps = [jnp.exp2((l - mx) * cexp) for l in logits]
            den = _tree(jnp.add, ps)
            r = pl.reciprocal(den, approx=True)
            inv = r * (2.0 - den * r)
            outs = []
            prev = None
            for j in range(NB):
                o = ps[0] * v_buf[j, pl.ds(base, RC), :]
                if prev is not None:
                    o = o + _fzero(prev)
                for w in range(1, W):
                    o = o + ps[w] * v_buf[j, pl.ds(base - dil * w, RC), :]
                prev = o
                outs.append(_pack(o * inv))
            ob = _butterfly(outs)
            for j in range(NB):
                a_buf[r0 // 2:(r0 + RC) // 2, LANES * j:LANES * (j + 1)] = ob[j]
            return _tree(jnp.bitwise_or, ob)

        def phase_b(t):
            dep = permute_kv(t)
            row0 = off_tab[0]
            for r0 in range(0, TM, RC):
                dep = attn_chunk(t, row0, r0, dep)
            lhs = load_lhs(t)
            accs = [None] * 7
            for c in range(NC):
                u0 = 3 * c * UR
                gu = _combine([_dot(lhs[i], rhs(wb_p, i, u0, KH)) for i in range(7)])
                hl = _lhs_combos(*[_silu(z[:, :CW]) * z[:, CW:] for z in gu])
                for i in range(7):
                    d = _dot(hl[i].astype(BF16), rhs(wb_p, i, u0 + KH, CW))
                    accs[i] = d if accs[i] is None else accs[i] + d
            ys = _combine(accs)
            a = pltpu.bitcast(a_buf[...], BF16).astype(F32)
            al = _lhs_combos(a[:TH, :KH], a[:TH, KH:], a[TH:, :KH], a[TH:, KH:])
            u0 = 3 * NC * UR
            ss = _combine([_dot(al[i].astype(BF16), rhs(wb_p, i, u0, KH)) for i in range(7)])
            for n in QORDER:
                rows, cols = quad_pos(t, n)
                o_buf[rows, cols] = (x_buf[rows, cols].astype(F32) + ss[n] * _silu(ys[n])).astype(BF16)
                o_cp(t, n).start()

        x_cp(0).start()
        for cp in wa_cps(0):
            cp.start()
        off_tab[0] = 0
        with scope("x0wait"):
            x_cp(0).wait()
        for n in range(1, x1at):
            for cp in wa_cps(n):
                cp.start()
        with scope("ln0"):
            layernorm(0, 0, keep_plain=True)
        phase_a0()

        def a_body(t, c):
            with scope("Await"):
                @pl.when(t + 1 < NT)
                def _():
                    x_cp(t + 1).wait()

                @pl.when(t + 2 < NT)
                def _():
                    x_cp(t + 2).start()
                for s in range(NS):
                    @pl.when(t == s + 2)
                    def _():
                        for cp in wb_cps(s):
                            cp.wait()
                for s in range(1, NS):
                    @pl.when(t == s)
                    def _():
                        for cp in wb_cps(s):
                            cp.start()
            with scope("A"):
                phase_a(t)
            return c
        jax.lax.fori_loop(1, NT, a_body, 0)

        def b_body(t, c):
            with scope("B"):
                phase_b(t)
            return c
        jax.lax.fori_loop(0, NT, b_body, 0)
        with scope("owait"):
            for t in range(NT):
                for n in range(4):
                    o_cp(t, n).wait()

    anyspec = pl.BlockSpec(memory_space=pl.ANY)
    out = pl.pallas_call(
        kernel,
        in_specs=[anyspec] * 6,
        out_specs=anyspec,
        out_shape=jax.ShapeDtypeStruct((S, D), A_x.dtype),
        scratch_shapes=[
            pltpu.VMEM((S, D), BF16), pltpu.VMEM((TH, D), U32), pltpu.VMEM((7 * S // 4, KH), U32),
            pltpu.VMEM((4, NH, KH), BF16), pltpu.VMEM((7 * NH // 2, KH), U32),
            pltpu.VMEM((4, RING * SR, KH), BF16), pltpu.VMEM((7 * NS * SR // 2, KH), U32),
            pltpu.VMEM((S // 2, 3 * D), U32),
            pltpu.VMEM((NB, TM + HALO, LANES), F32), pltpu.VMEM((NB, TM + HALO, LANES), F32),
            pltpu.VMEM((TH, D), U32), pltpu.VMEM((S, D), BF16), pltpu.SMEM((1,), jnp.int32),
            pltpu.SemaphoreType.DMA((NT,)), pltpu.SemaphoreType.DMA((NSUB,)),
            pltpu.SemaphoreType.DMA((NS,)), pltpu.SemaphoreType.DMA((4 * NT,)),
        ],
        compiler_params=pltpu.CompilerParams(vmem_limit_bytes=124 * 1024 * 1024, disable_bounds_checks=True,
                                             disable_semaphore_checks=True),
    )(A_x.reshape(S, D), A_wqkv.reshape(2, KH, 3 * D), A_wo.reshape(2, KH, D),
      B_w_gate.reshape(2, KH, F), B_w_up.reshape(2, KH, F), B_w_down.reshape(2, FH, D))
    return out.reshape(B, S, D)


@jax.jit
def pallas_recurrent_scan__sliding_local_dilated__swiglu_ffn__prompt_kernel(A_x, A_wqkv, A_wo, B_x, B_w_gate, B_w_up, B_w_down):
    return build(A_x, A_wqkv, A_wo, B_x, B_w_gate, B_w_up, B_w_down)
```

```python
import contextlib
import math
import jax
import jax.numpy as jnp
import jax.experimental.pallas as pl
import jax.experimental.pallas.tpu as pltpu

F32 = jnp.float32
BF16 = jnp.bfloat16
U32 = jnp.uint32
HALO = 16
LANES = 128
QORDER = (2, 1, 3, 0)


def _butterfly(blocks):
    lane = jax.lax.broadcasted_iota(jnp.int32, blocks[0].shape, 1)
    for beta in (1, 2, 4):
        hi = (lane & (4 * beta)) != 0
        new = list(blocks)
        for j0 in range(8):
            if j0 & beta:
                continue
            j1 = j0 | beta
            new[j0] = jnp.where(hi, pltpu.roll(blocks[j1], 4 * beta, 1), blocks[j0])
            new[j1] = jnp.where(hi, blocks[j1], pltpu.roll(blocks[j0], LANES - 4 * beta, 1))
        blocks = new
    return blocks


def _opaque_zero(v):
    s = jnp.uint32(16)
    return jax.lax.shift_right_logical(jax.lax.shift_right_logical(v, s), s)


def _fzero(v):
    return pltpu.bitcast(_opaque_zero(pltpu.bitcast(v, U32)), F32)


def _silu(x):
    hx = 0.5 * x
    return hx * (1.0 + jnp.tanh(hx))


def _tree(op, xs):
    xs = list(xs)
    while len(xs) > 1:
        xs = [op(xs[i], xs[i + 1]) if i + 1 < len(xs) else xs[i] for i in range(0, len(xs), 2)]
    return xs[0]


def _lhs_combos(a11, a12, a21, a22):
    return [a11 + a22, a21 + a22, a11, a22, a11 + a12, a21 - a11, a12 - a22]


def _combine(m):
    return m[0] + m[3] - m[4] + m[6], m[2] + m[4], m[1] + m[3], m[0] - m[1] + m[2] + m[5]


def _pack(y):
    return pltpu.bitcast(y.astype(BF16), U32)


def _dot(a, b):
    return jnp.dot(a, b, preferred_element_type=F32)


def build(A_x, A_wqkv, A_wo, B_x, B_w_gate, B_w_up, B_w_down,
          subs=(128, 128, 256, 256, 256, 256, 128, 128), x1at=6, ln1=(6, 7), ln1chain=2, pchain=3, lnchain=1,
          PR=16, CG=256,  pfirst=True, sideat=3, morder=(0, 1, 2, 3, 4, 5, 6), wnd=0, lnp=1, dorder=(1, 3, 6, 0, 2, 4, 5), swp=False, dgrp=1, gate=False,  wchain=2, p0chain=2, scopes=False):
    scope = jax.named_scope if scopes else (lambda name: contextlib.nullcontext())
    B, S, D = A_x.shape
    F = B_w_gate.shape[1]
    H = 32
    Dh = D // H
    W, dil = 8, 2
    scale = Dh ** -0.5
    NB = D // LANES
    TM = 256
    NT = S // TM
    RC = 16
    TH = TM // 2
    TQ = TM // 4
    KH = D // 2
    FH = F // 2
    NH = 3 * D // 2
    CW = KH // 2
    NC = FH // CW
    UR = 256
    NU = 3 * NC + 2
    UPS = 4
    NS = NT - 2
    SR = UPS * UR
    RING = 3
    assert NS * UPS >= NU and sum(subs) == NH
    NSUB = len(subs)
    sub_off = [sum(subs[:n]) for n in range(NSUB)]
    assert all(o // KH == (o + s - 1) // KH for o, s in zip(sub_off, subs))

    def kernel(x_hbm, wqkv_hbm, wo_hbm, wg_hbm, wu_hbm, wd_hbm, o_hbm,
               x_buf, xn0, xs_buf, wa, wa_p, wb, wb_p, qkv_raw, k_buf, v_buf, a_buf, o_buf, off_tab,
               x_sem, wa_sem, wb_sem, o_sem):
        def tile_rows(t):
            return pl.ds(pl.multiple_of(t * TM, TM), TM)

        def x_cp(t):
            return pltpu.make_async_copy(x_hbm.at[tile_rows(t), :], x_buf.at[tile_rows(t), :], x_sem.at[t])

        def quad_pos(t, n):
            i, j = divmod(n, 2)
            return pl.ds(pl.multiple_of(t * TM + i * TH, TH), TH), pl.ds(j * KH, KH)

        def o_cp(t, n):
            rows, cols = quad_pos(t, n)
            return pltpu.make_async_copy(o_buf.at[rows, cols], o_hbm.at[rows, cols], o_sem.at[4 * t + n])

        def sub_pos(n):
            u, c = divmod(sub_off[n], KH)
            return pl.ds(u * KH, KH), pl.ds(c, subs[n])

        def wa_cps(n):
            rows, cols = sub_pos(n)
            return [pltpu.make_async_copy(wqkv_hbm.at[:, :, pl.ds(j * NH + sub_off[n], subs[n])],
                                          wa.at[pl.ds(2 * j, 2), rows, cols], wa_sem.at[n]) for j in range(2)]

        def wb_cps(s):
            cps = []
            for u in range(s * UPS, min((s + 1) * UPS, NU)):
                rows = pl.ds((s % RING) * SR + (u - s * UPS) * UR, UR)
                c, part = divmod(u, 3)
                for j in range(2):
                    dst = wb.at[pl.ds(2 * j, 2), rows, :]
                    if c == NC:
                        srcs = [(wo_hbm.at[:, pl.ds(part * UR, UR), pl.ds(j * KH, KH)], dst)]
                    elif part == 2:
                        srcs = [(wd_hbm.at[:, pl.ds(c * CW, CW), pl.ds(j * KH, KH)], dst)]
                    else:
                        srcs = [(w.at[:, pl.ds(part * UR, UR), pl.ds(j * FH + c * CW, CW)],
                                 wb.at[pl.ds(2 * j, 2), rows, pl.ds(n * CW, CW)])
                                for n, w in enumerate((wg_hbm, wu_hbm))]
                    cps += [pltpu.make_async_copy(a, b, wb_sem.at[s]) for a, b in srcs]
            return cps

        def layernorm(t, nchain, keep_plain=False, dep0=None, r_lo=0, r_hi=TH):
            deps = [] if dep0 is None else [dep0] * nchain
            g = 16
            for r in range(r_lo, r_hi, g):
                x = jnp.concatenate(
                    [x_buf[pl.ds(pl.multiple_of(t * TM + h * TH + r, g), g), :].astype(F32) for h in range(2)], axis=0)
                m = jnp.mean(x, axis=-1, keepdims=True)
                if nchain and len(deps) >= nchain:
                    m = m + pltpu.bitcast(_opaque_zero(deps[-nchain]), F32)
                xc = x - m
                var = jnp.mean(xc * xc, axis=-1, keepdims=True)
                rs = jax.lax.rsqrt(var + 1e-5)
                if gate and nchain:
                    allz = _fzero(_tree(jnp.add, [rs[q:q + 8] for q in range(0, 2 * g, 8)]))
                    rs = rs + jnp.concatenate([allz] * (2 * g // 8), axis=0)
                npiece = lnp if nchain else 1
                cw = KH // npiece
                for p in range(npiece):
                    if p > 0:
                        z = pltpu.roll(_fzero(last), 1, 1)[:, 0:1]
                        rs = rs + jnp.concatenate([z] * (2 * g // 8), axis=0)
                    cl, cr = slice(p * cw, (p + 1) * cw), slice(KH + p * cw, KH + (p + 1) * cw)
                    xl, xr = xc[:, cl] * rs, xc[:, cr] * rs
                    if keep_plain:
                        for h in range(2):
                            xn0[h * TQ + r // 2:h * TQ + (r + g) // 2, cl] = _pack(xl[h * g:(h + 1) * g])
                            xn0[h * TQ + r // 2:h * TQ + (r + g) // 2, cr] = _pack(xr[h * g:(h + 1) * g])
                    combos = _lhs_combos(xl[:g], xr[:g], xl[g:], xr[g:])
                    for n in range(7):
                        xs_buf[pl.ds(pl.multiple_of(n * (S // 4) + t * TQ + r // 2, g // 2), g // 2), cl] = _pack(combos[n])
                    last = combos[6][0:8, cw - LANES:cw]
                deps.append(pltpu.bitcast(xr[:, cw - 1:cw], U32))
            return pltpu.bitcast(last, U32)

        def prep(w, row0, nrows, c0, ncols, dst, dst_row0, nchain, dep0=None, nd=0):
            deps = [] if dep0 is None else [dep0] * nchain
            plane = dst.shape[0] // 7
            half0 = dst_row0 // 2
            cg = min(CG, ncols)
            for r in range(0, nrows, PR):
                rows = pl.ds(pl.multiple_of(row0 + r, PR), PR)
                for c in range(c0, c0 + ncols, cg):
                    cols = pl.ds(c, cg)
                    b11, b21, b12, b22 = [w[s, rows, cols].astype(F32) for s in range(4)]
                    if nchain and len(deps) >= nchain:
                        z = _fzero(deps[-nchain])
                        if nd == 0:
                            z = pltpu.roll(z, 1, 1)
                        for _ in range(nd):
                            z = jnp.tanh(z)
                        z = jnp.concatenate([jnp.concatenate([z] * (cg // LANES), axis=1)] * (PR // 8), axis=0)
                        b11 = b11 + z
                        b22 = b22 + z
                    outs = [b11 + b22, b11, b12 - b22, b21 - b11, b22, b11 + b12, b21 + b22]
                    deps.append(outs[6][PR - 8:, cg - LANES:])
                    for i in range(7):
                        dst[pl.ds(pl.multiple_of(half0 + (i * plane + r // 2), PR // 2), PR // 2), cols] = _pack(outs[i])
            return deps[-1]

        def rhs(dst, i, row0, nrows):
            plane = dst.shape[0] // 7
            return pltpu.bitcast(dst[i * plane + row0 // 2:i * plane + (row0 + nrows) // 2, :], BF16)

        def load_lhs(t):
            return [pltpu.bitcast(xs_buf[pl.ds(pl.multiple_of(n * (S // 4) + t * TQ, TQ), TQ), :], BF16)
                    for n in range(7)]

        def phase_a0():
            for n in range(NSUB + 1):
                if n < NSUB:
                    with scope(f"wawait{n}"):
                        for cp in wa_cps(n):
                            cp.wait()
                if n == ln1[0]:
                    with scope("x1wait"):
                        x_cp(1).wait()
                if n == 0:
                    x_cp(1).start()
                if n == 1:
                    for m in range(x1at, NSUB):
                        for cp in wa_cps(m):
                            cp.start()
                if n == NSUB - 3:
                    x_cp(2).start()
                if n == NSUB - 2:
                    for cp in wb_cps(0):
                        cp.start()
                if n in ln1:
                    k = ln1.index(n)
                    layernorm(1, ln1chain, r_lo=k * TH // len(ln1), r_hi=(k + 1) * TH // len(ln1))
                if n > 0:
                    rows, cols = sub_pos(n - 1)
                    prep(wa, rows.start, KH, cols.start, cols.size, wa_p, rows.start, 0 if n == NSUB else (p0chain if subs[n] >= 256 else 2 * p0chain))
                if n < NSUB:
                    rows, cols = sub_pos(n)
                    xn = pltpu.bitcast(xn0[...], BF16)
                    for j in range(2):
                        wj = jnp.concatenate([wa[2 * j, rows, cols], wa[2 * j + 1, rows, cols]], axis=0)
                        c0 = j * NH + sub_off[n]
                        qkv_raw[0:TH, c0:c0 + subs[n]] = _pack(_dot(xn, wj))

        def phase_a(t):
            def side():
                s = jnp.where(t >= 2, t - 2, NS - 1)
                tn = jnp.minimum(t + 1, NT - 1)
                if pfirst:
                    prep(wb, ((t + 1) % RING) * SR, SR, 0, KH, wb_p, s * SR, wchain, nd=wnd)
                layernorm(tn, lnchain)
                if not pfirst:
                    prep(wb, ((t + 1) % RING) * SR, SR, 0, KH, wb_p, s * SR, wchain, nd=wnd)

            lhs = load_lhs(t)
            for u in range(NH // KH):
                if u == sideat:
                    side()
                ms = [None] * 7
                for i in morder:
                    ms[i] = _dot(lhs[i], rhs(wa_p, i, u * KH, KH))
                quads = _combine(ms)
                for n in QORDER:
                    i, j = divmod(n, 2)
                    qkv_raw[pl.ds(pl.multiple_of(t * TH + i * TQ, TQ), TQ), j * NH + u * KH:j * NH + (u + 1) * KH] = (
                        _pack(quads[n]))
            if sideat >= NH // KH:
                side()

        def permute_kv(t):
            deps = []
            for r in range(-HALO, TM, 16):
                src0 = jnp.maximum(t * TH + r // 2, 0) if r < 0 else t * TH + r // 2
                for part, dst in ((1, k_buf), (2, v_buf)):
                    src_rows = pl.ds(pl.multiple_of(src0, 8), 8)
                    blocks = [qkv_raw[src_rows, part * D + LANES * j:part * D + LANES * (j + 1)] for j in range(NB)]
                    if len(deps) >= pchain:
                        zero = _opaque_zero(deps[-pchain])
                        blocks = [b | zero for b in blocks]
                    blocks = _butterfly(blocks)
                    deps.append(blocks[NB - 1])
                    for j in range(NB):
                        dst[j, HALO + r:HALO + r + 16, :] = pltpu.bitcast(blocks[j], BF16).astype(F32)
            return _tree(jnp.bitwise_or, deps[-pchain:])

        lane = jax.lax.broadcasted_iota(jnp.int32, (RC, LANES), 1)
        odd = (lane & 1) == 1
        hi2 = (lane & 2) == 2
        rowi = jax.lax.broadcasted_iota(jnp.int32, (RC, LANES), 0)
        cexp = scale * math.log2(math.e)

        def attn_chunk(t, row0, r0, dep):
            zero = _opaque_zero(dep)
            qrows = pl.ds(pl.multiple_of(t * TH + r0 // 2, 8), RC // 2)
            qb = _butterfly([qkv_raw[qrows, LANES * j:LANES * (j + 1)] | zero for j in range(NB)])
            qs = [pltpu.bitcast(b, BF16).astype(F32) for b in qb]
            base = row0 + (HALO + r0)
            logits = []
            prev = None
            for w in range(W):
                acc = qs[0] * k_buf[0, pl.ds(base - dil * w, RC), :]
                if prev is not None:
                    acc = acc + _fzero(prev)
                for j in range(1, NB):
                    acc = acc + qs[j] * k_buf[j, pl.ds(base - dil * w, RC), :]
                prev = acc
                acc = acc + jnp.where(odd, pltpu.roll(acc, 1, 1), pltpu.roll(acc, LANES - 1, 1))
                acc = acc + jnp.where(hi2, pltpu.roll(acc, 2, 1), pltpu.roll(acc, LANES - 2, 1))
                if w > 0 and r0 < dil * w:
                    pos = rowi + (t * TM + r0 - dil * w)
                    acc = jnp.where(pos >= 0, acc, -1e9 / scale)
                logits.append(acc)
            mx = _tree(jnp.maximum, logits)
            ps = [jnp.exp2((l - mx) * cexp) for l in logits]
            den = _tree(jnp.add, ps)
            r = pl.reciprocal(den, approx=True)
            inv = r * (2.0 - den * r)
            outs = []
            prev = None
            for j in range(NB):
                o = ps[0] * v_buf[j, pl.ds(base, RC), :]
                if prev is not None:
                    o = o + _fzero(prev)
                for w in range(1, W):
                    o = o + ps[w] * v_buf[j, pl.ds(base - dil * w, RC), :]
                prev = o
                outs.append(_pack(o * inv))
            ob = _butterfly(outs)
            for j in range(NB):
                a_buf[r0 // 2:(r0 + RC) // 2, LANES * j:LANES * (j + 1)] = ob[j]
            return _tree(jnp.bitwise_or, ob)

        def phase_b(t):
            dep = permute_kv(t)
            row0 = off_tab[0]
            for r0 in range(0, TM, RC):
                dep = attn_chunk(t, row0, r0, dep)
            lhs = load_lhs(t)
            accs = [None] * 7

            def hidden(c):
                gu = _combine([_dot(lhs[i], rhs(wb_p, i, 3 * c * UR, KH)) for i in range(7)])
                return [h.astype(BF16) for h in _lhs_combos(*[_silu(z[:, :CW]) * z[:, CW:] for z in gu])]

            def down(cs, hls):
                for i in dorder:
                    l = jnp.concatenate([hl[i] for hl in hls], axis=1)
                    w = jnp.concatenate([rhs(wb_p, i, 3 * c * UR + KH, CW) for c in cs], axis=0)
                    d = _dot(l, w)
                    accs[i] = d if accs[i] is None else accs[i] + d

            pend = []
            for c in range(NC):
                hl = hidden(c)
                if not swp:
                    pend.append((c, hl))
                if len(pend) >= dgrp:
                    down(*zip(*pend))
                    pend = []
                if swp:
                    pend.append((c, hl))
            if pend:
                down(*zip(*pend))
            ys = _combine(accs)
            a = pltpu.bitcast(a_buf[...], BF16).astype(F32)
            al = _lhs_combos(a[:TH, :KH], a[:TH, KH:], a[TH:, :KH], a[TH:, KH:])
            u0 = 3 * NC * UR
            ss = _combine([_dot(al[i].astype(BF16), rhs(wb_p, i, u0, KH)) for i in range(7)])
            for n in QORDER:
                rows, cols = quad_pos(t, n)
                o_buf[rows, cols] = (x_buf[rows, cols].astype(F32) + ss[n] * _silu(ys[n])).astype(BF16)
                o_cp(t, n).start()

        x_cp(0).start()
        for cp in wa_cps(0):
            cp.start()
        off_tab[0] = 0
        with scope("x0wait"):
            x_cp(0).wait()
        for n in range(1, x1at):
            for cp in wa_cps(n):
                cp.start()
        with scope("ln0"):
            layernorm(0, 0, keep_plain=True)
        phase_a0()

        def a_body(t, c):
            with scope("Await"):
                @pl.when(t + 1 < NT)
                def _():
                    x_cp(t + 1).wait()

                @pl.when(t + 2 < NT)
                def _():
                    x_cp(t + 2).start()
                for s in range(NS):
                    @pl.when(t == s + 2)
                    def _():
                        for cp in wb_cps(s):
                            cp.wait()
                for s in range(1, NS):
                    @pl.when(t == s)
                    def _():
                        for cp in wb_cps(s):
                            cp.start()
            with scope("A"):
                phase_a(t)
            return c
        jax.lax.fori_loop(1, NT, a_body, 0)

        def b_body(t, c):
            with scope("B"):
                phase_b(t)
            return c
        jax.lax.fori_loop(0, NT, b_body, 0)
        with scope("owait"):
            for t in range(NT):
                for n in range(4):
                    o_cp(t, n).wait()

    anyspec = pl.BlockSpec(memory_space=pl.ANY)
    out = pl.pallas_call(
        kernel,
        in_specs=[anyspec] * 6,
        out_specs=anyspec,
        out_shape=jax.ShapeDtypeStruct((S, D), A_x.dtype),
        scratch_shapes=[
            pltpu.VMEM((S, D), BF16), pltpu.VMEM((TH, D), U32), pltpu.VMEM((7 * S // 4, KH), U32),
            pltpu.VMEM((4, NH, KH), BF16), pltpu.VMEM((7 * NH // 2, KH), U32),
            pltpu.VMEM((4, RING * SR, KH), BF16), pltpu.VMEM((7 * NS * SR // 2, KH), U32),
            pltpu.VMEM((S // 2, 3 * D), U32),
            pltpu.VMEM((NB, TM + HALO, LANES), F32), pltpu.VMEM((NB, TM + HALO, LANES), F32),
            pltpu.VMEM((TH, D), U32), pltpu.VMEM((S, D), BF16), pltpu.SMEM((1,), jnp.int32),
            pltpu.SemaphoreType.DMA((NT,)), pltpu.SemaphoreType.DMA((NSUB,)),
            pltpu.SemaphoreType.DMA((NS,)), pltpu.SemaphoreType.DMA((4 * NT,)),
        ],
        compiler_params=pltpu.CompilerParams(vmem_limit_bytes=124 * 1024 * 1024, disable_bounds_checks=True,
                                             disable_semaphore_checks=True),
    )(A_x.reshape(S, D), A_wqkv.reshape(2, KH, 3 * D), A_wo.reshape(2, KH, D),
      B_w_gate.reshape(2, KH, F), B_w_up.reshape(2, KH, F), B_w_down.reshape(2, FH, D))
    return out.reshape(B, S, D)


@jax.jit
def pallas_recurrent_scan__sliding_local_dilated__swiglu_ffn__prompt_kernel(A_x, A_wqkv, A_wo, B_x, B_w_gate, B_w_up, B_w_down):
    return build(A_x, A_wqkv, A_wo, B_x, B_w_gate, B_w_up, B_w_down)
```

```python
import contextlib
import math
import jax
import jax.numpy as jnp
import jax.experimental.pallas as pl
import jax.experimental.pallas.tpu as pltpu

F32 = jnp.float32
BF16 = jnp.bfloat16
U32 = jnp.uint32
HALO = 16
LANES = 128
QORDER = (2, 1, 3, 0)


def _butterfly(blocks):
    lane = jax.lax.broadcasted_iota(jnp.int32, blocks[0].shape, 1)
    for beta in (1, 2, 4):
        hi = (lane & (4 * beta)) != 0
        new = list(blocks)
        for j0 in range(8):
            if j0 & beta:
                continue
            j1 = j0 | beta
            new[j0] = jnp.where(hi, pltpu.roll(blocks[j1], 4 * beta, 1), blocks[j0])
            new[j1] = jnp.where(hi, blocks[j1], pltpu.roll(blocks[j0], LANES - 4 * beta, 1))
        blocks = new
    return blocks


def _opaque_zero(v):
    s = jnp.uint32(16)
    return jax.lax.shift_right_logical(jax.lax.shift_right_logical(v, s), s)


def _fzero(v):
    return pltpu.bitcast(_opaque_zero(pltpu.bitcast(v, U32)), F32)


def _silu(x):
    hx = 0.5 * x
    return hx * (1.0 + jnp.tanh(hx))


def _tree(op, xs):
    xs = list(xs)
    while len(xs) > 1:
        xs = [op(xs[i], xs[i + 1]) if i + 1 < len(xs) else xs[i] for i in range(0, len(xs), 2)]
    return xs[0]


def _lhs_combos(a11, a12, a21, a22):
    return [a11 + a22, a21 + a22, a11, a22, a11 + a12, a21 - a11, a12 - a22]


def _combine(m):
    return m[0] + m[3] - m[4] + m[6], m[2] + m[4], m[1] + m[3], m[0] - m[1] + m[2] + m[5]


def _pack(y):
    return pltpu.bitcast(y.astype(BF16), U32)


def _dot(a, b):
    return jnp.dot(a, b, preferred_element_type=F32)


def build(A_x, A_wqkv, A_wo, B_x, B_w_gate, B_w_up, B_w_down,
          subs=(128, 128, 256, 256, 256, 256, 128, 128), x1at=6, ln1=(6, 7), ln1chain=2, pchain=3, lnchain=1,
          PR=16, CG=256,  pfirst=True, late_starts={1: (3, 4), 2: (5,)}, uorder=(0, 1, 2), dcol=0, lnskew=68, sideat=3, morder=(0, 1, 2, 3, 4, 5, 6), wnd=0, lnp=1, dorder=(1, 3, 6, 0, 2, 4, 5), swp=False, dgrp=1, gate=True,  wchain=2, p0chain=2, scopes=False):
    scope = jax.named_scope if scopes else (lambda name: contextlib.nullcontext())
    B, S, D = A_x.shape
    F = B_w_gate.shape[1]
    H = 32
    Dh = D // H
    W, dil = 8, 2
    scale = Dh ** -0.5
    NB = D // LANES
    TM = 256
    NT = S // TM
    RC = 16
    TH = TM // 2
    TQ = TM // 4
    KH = D // 2
    FH = F // 2
    NH = 3 * D // 2
    CW = KH // 2
    NC = FH // CW
    UR = 256
    NU = 3 * NC + 2
    UPS = 4
    NS = NT - 2
    SR = UPS * UR
    assert NS * UPS >= NU and sum(subs) == NH
    NSUB = len(subs)
    sub_off = [sum(subs[:n]) for n in range(NSUB)]
    assert all(o // KH == (o + s - 1) // KH for o, s in zip(sub_off, subs))

    def kernel(x_hbm, wqkv_hbm, wo_hbm, wg_hbm, wu_hbm, wd_hbm, o_hbm,
               x_buf, xn0, xs_buf, wa, wb, wa_p, wb_p, qkv_raw, k_buf, v_buf, a_buf, o_buf, off_tab,
               x_sem, wa_sem, wb_sem, o_sem):
        def tile_rows(t):
            return pl.ds(pl.multiple_of(t * TM, TM), TM)

        xgroups = ((0, 1), (1, 2), (2, 4), (4, NT))

        def x_cp(n):
            rows = pl.ds(xgroups[n][0] * TM, (xgroups[n][1] - xgroups[n][0]) * TM)
            return pltpu.make_async_copy(x_hbm.at[rows, :], x_buf.at[rows, :], x_sem.at[n])

        def quad_pos(t, n):
            i, j = divmod(n, 2)
            return pl.ds(pl.multiple_of(t * TM + i * TH, TH), TH), pl.ds(j * KH, KH)

        def o_cp(t, n):
            rows, cols = quad_pos(t, n)
            return pltpu.make_async_copy(o_buf.at[rows, cols], o_hbm.at[rows, cols], o_sem.at[4 * t + n])

        def sub_pos(n):
            u, c = divmod(sub_off[n], KH)
            return pl.ds(u * KH, KH), pl.ds(c, subs[n])

        def wa_cps(n):
            rows, cols = sub_pos(n)
            return [pltpu.make_async_copy(wqkv_hbm.at[:, :, pl.ds(j * NH + sub_off[n], subs[n])],
                                          wa.at[pl.ds(2 * j, 2), rows, cols], wa_sem.at[n]) for j in range(2)]

        def wb_cps(s):
            cps = []
            u, end = s * UPS, min((s + 1) * UPS, NU)
            while u < end:
                c, part = divmod(u, 3)
                nu = 2 if (part == 0 and u + 1 < end) else 1
                rows = pl.ds(u * UR, nu * UR)
                for j in range(2):
                    dst = wb.at[pl.ds(2 * j, 2), rows, :]
                    if c == NC:
                        srcs = [(wo_hbm.at[:, pl.ds(part * UR, nu * UR), pl.ds(j * KH, KH)], dst)]
                    elif part == 2:
                        srcs = [(wd_hbm.at[:, pl.ds(c * CW, CW), pl.ds(j * KH, KH)], dst)]
                    else:
                        srcs = [(w.at[:, pl.ds(part * UR, nu * UR), pl.ds(j * FH + c * CW, CW)],
                                 wb.at[pl.ds(2 * j, 2), rows, pl.ds(n * CW, CW)])
                                for n, w in enumerate((wg_hbm, wu_hbm))]
                    cps += [pltpu.make_async_copy(a, b, wb_sem.at[s]) for a, b in srcs]
                u += nu
            return cps

        def layernorm(t, nchain, keep_plain=False, dep0=None, r_lo=0, r_hi=TH):
            deps = [] if dep0 is None else [dep0] * nchain
            g = 16
            for r in range(r_lo, r_hi, g):
                x = jnp.concatenate(
                    [x_buf[pl.ds(pl.multiple_of(t * TM + h * TH + r, g), g), :].astype(F32) for h in range(2)], axis=0)
                m = jnp.mean(x, axis=-1, keepdims=True)
                if nchain and len(deps) >= nchain:
                    m = m + pltpu.bitcast(_opaque_zero(deps[-nchain]), F32)
                xc = x - m
                var = jnp.mean(xc * xc, axis=-1, keepdims=True)
                rs = jax.lax.rsqrt(var + 1e-5)
                if gate and nchain:
                    allz = _fzero(_tree(jnp.add, [rs[q:q + 8] for q in range(0, 2 * g, 8)]))
                    rs = rs + jnp.concatenate([allz] * (2 * g // 8), axis=0)
                npiece = lnp if nchain else 1
                cw = KH // npiece
                for p in range(npiece):
                    if p > 0:
                        z = pltpu.roll(_fzero(last), 1, 1)[:, 0:1]
                        rs = rs + jnp.concatenate([z] * (2 * g // 8), axis=0)
                    cl, cr = slice(p * cw, (p + 1) * cw), slice(KH + p * cw, KH + (p + 1) * cw)
                    xl, xr = xc[:, cl] * rs, xc[:, cr] * rs
                    if keep_plain:
                        for h in range(2):
                            xn0[h * TQ + r // 2:h * TQ + (r + g) // 2, cl] = _pack(xl[h * g:(h + 1) * g])
                            xn0[h * TQ + r // 2:h * TQ + (r + g) // 2, cr] = _pack(xr[h * g:(h + 1) * g])
                    combos = _lhs_combos(xl[:g], xr[:g], xl[g:], xr[g:])
                    for n in range(7):
                        xs_buf[pl.ds(pl.multiple_of(n * (S // 4) + t * TQ + r // 2, g // 2), g // 2), cl] = _pack(combos[n])
                    last = combos[6][0:8, cw - LANES:cw]
                deps.append(pltpu.bitcast(xr[:, cw - 1:cw], U32))
            return pltpu.bitcast(last, U32)

        def prep(w, row0, nrows, c0, ncols, dst, dst_row0, nchain, dep0=None, nd=0, live=None):
            deps = [] if dep0 is None else [dep0] * nchain
            plane = dst.shape[0] // 7
            half0 = dst_row0 // 2
            cg = min(CG, ncols)
            for r in range(0, nrows, PR):
                src0 = row0 + r if live is None else jnp.where(live, row0 + r, NS * SR)
                rows = pl.ds(pl.multiple_of(src0, PR), PR)
                for c in range(c0, c0 + ncols, cg):
                    cols = pl.ds(c, cg)
                    b11, b21, b12, b22 = [w[s, rows, cols].astype(F32) for s in range(4)]
                    if nchain and len(deps) >= nchain:
                        z = _fzero(deps[-nchain])
                        if nd == 0:
                            z = pltpu.roll(z, 1, 1)
                        for _ in range(nd):
                            z = jnp.tanh(z)
                        z = jnp.concatenate([jnp.concatenate([z] * (cg // LANES), axis=1)] * (PR // 8), axis=0)
                        b11 = b11 + z
                        b22 = b22 + z
                    outs = [b11 + b22, b11, b12 - b22, b21 - b11, b22, b11 + b12, b21 + b22]
                    deps.append(outs[dcol * 6][PR - 8:, cg - LANES:])
                    for i in range(7):
                        dst[pl.ds(pl.multiple_of(half0 + (i * plane + r // 2), PR // 2), PR // 2), cols] = _pack(outs[i])
            return deps

        def rhs(dst, i, row0, nrows):
            plane = dst.shape[0] // 7
            return pltpu.bitcast(dst[i * plane + row0 // 2:i * plane + (row0 + nrows) // 2, :], BF16)

        def load_lhs(t):
            return [pltpu.bitcast(xs_buf[pl.ds(pl.multiple_of(n * (S // 4) + t * TQ, TQ), TQ), :], BF16)
                    for n in range(7)]

        def phase_a0():
            for n in range(NSUB + 1):
                if n < NSUB:
                    with scope(f"wawait{n}"):
                        for cp in wa_cps(n):
                            cp.wait()
                if n == ln1[0]:
                    with scope("x1wait"):
                        x_cp(1).wait()
                if n in ln1:
                    k = ln1.index(n)
                    layernorm(1, ln1chain, r_lo=k * TH // len(ln1), r_hi=(k + 1) * TH // len(ln1))
                if n > 0:
                    rows, cols = sub_pos(n - 1)
                    prep(wa, rows.start, KH, cols.start, cols.size, wa_p, rows.start, 0 if n == NSUB else (p0chain if subs[n] >= 256 else 2 * p0chain))
                if n < NSUB:
                    rows, cols = sub_pos(n)
                    xn = pltpu.bitcast(xn0[...], BF16)
                    for j in range(2):
                        wj = jnp.concatenate([wa[2 * j, rows, cols], wa[2 * j + 1, rows, cols]], axis=0)
                        c0 = j * NH + sub_off[n]
                        qkv_raw[0:TH, c0:c0 + subs[n]] = _pack(_dot(xn, wj))
                for s in late_starts.get(n, ()):
                    for cp in wb_cps(s):
                        cp.start()

        def phase_a(t):
            def side():
                s = jnp.where(t >= 2, t - 2, NS - 1)
                tn = jnp.minimum(t + 1, NT - 1)
                d0 = None
                if pfirst:
                    pd = prep(wb, s * SR, SR, 0, KH, wb_p, s * SR, wchain, nd=wnd, live=t >= 2)
                    if lnskew:
                        d0 = pltpu.bitcast(jnp.concatenate([pd[lnskew]] * 4, axis=0)[:, 0:1], U32)
                layernorm(tn, lnchain, dep0=d0)
                if not pfirst:
                    prep(wb, s * SR, SR, 0, KH, wb_p, s * SR, wchain, nd=wnd, live=t >= 2)

            lhs = load_lhs(t)
            for u in uorder:
                if u == sideat:
                    side()
                ms = [None] * 7
                for i in morder:
                    ms[i] = _dot(lhs[i], rhs(wa_p, i, u * KH, KH))
                quads = _combine(ms)
                for n in QORDER:
                    i, j = divmod(n, 2)
                    qkv_raw[pl.ds(pl.multiple_of(t * TH + i * TQ, TQ), TQ), j * NH + u * KH:j * NH + (u + 1) * KH] = (
                        _pack(quads[n]))
            if sideat >= NH // KH:
                side()

        def permute_kv(t):
            deps = []
            for r in range(-HALO, TM, 16):
                src0 = jnp.maximum(t * TH + r // 2, 0) if r < 0 else t * TH + r // 2
                for part, dst in ((1, k_buf), (2, v_buf)):
                    src_rows = pl.ds(pl.multiple_of(src0, 8), 8)
                    blocks = [qkv_raw[src_rows, part * D + LANES * j:part * D + LANES * (j + 1)] for j in range(NB)]
                    if len(deps) >= pchain:
                        zero = _opaque_zero(deps[-pchain])
                        blocks = [b | zero for b in blocks]
                    blocks = _butterfly(blocks)
                    deps.append(blocks[NB - 1])
                    for j in range(NB):
                        dst[j, HALO + r:HALO + r + 16, :] = pltpu.bitcast(blocks[j], BF16).astype(F32)
            return _tree(jnp.bitwise_or, deps[-pchain:])

        lane = jax.lax.broadcasted_iota(jnp.int32, (RC, LANES), 1)
        odd = (lane & 1) == 1
        hi2 = (lane & 2) == 2
        rowi = jax.lax.broadcasted_iota(jnp.int32, (RC, LANES), 0)
        cexp = scale * math.log2(math.e)

        def attn_chunk(t, row0, r0, dep):
            zero = _opaque_zero(dep)
            qrows = pl.ds(pl.multiple_of(t * TH + r0 // 2, 8), RC // 2)
            qb = _butterfly([qkv_raw[qrows, LANES * j:LANES * (j + 1)] | zero for j in range(NB)])
            qs = [pltpu.bitcast(b, BF16).astype(F32) for b in qb]
            base = row0 + (HALO + r0)
            logits = []
            prev = None
            for w in range(W):
                acc = qs[0] * k_buf[0, pl.ds(base - dil * w, RC), :]
                if prev is not None:
                    acc = acc + _fzero(prev)
                for j in range(1, NB):
                    acc = acc + qs[j] * k_buf[j, pl.ds(base - dil * w, RC), :]
                prev = acc
                acc = acc + jnp.where(odd, pltpu.roll(acc, 1, 1), pltpu.roll(acc, LANES - 1, 1))
                acc = acc + jnp.where(hi2, pltpu.roll(acc, 2, 1), pltpu.roll(acc, LANES - 2, 1))
                if w > 0 and r0 < dil * w:
                    pos = rowi + (t * TM + r0 - dil * w)
                    acc = jnp.where(pos >= 0, acc, -1e9 / scale)
                logits.append(acc)
            mx = _tree(jnp.maximum, logits)
            ps = [jnp.exp2((l - mx) * cexp) for l in logits]
            den = _tree(jnp.add, ps)
            r = pl.reciprocal(den, approx=True)
            inv = r * (2.0 - den * r)
            outs = []
            prev = None
            for j in range(NB):
                o = ps[0] * v_buf[j, pl.ds(base, RC), :]
                if prev is not None:
                    o = o + _fzero(prev)
                for w in range(1, W):
                    o = o + ps[w] * v_buf[j, pl.ds(base - dil * w, RC), :]
                prev = o
                outs.append(_pack(o * inv))
            ob = _butterfly(outs)
            for j in range(NB):
                a_buf[r0 // 2:(r0 + RC) // 2, LANES * j:LANES * (j + 1)] = ob[j]
            return _tree(jnp.bitwise_or, ob)

        def phase_b(t):
            dep = permute_kv(t)
            row0 = off_tab[0]
            for r0 in range(0, TM, RC):
                dep = attn_chunk(t, row0, r0, dep)
            lhs = load_lhs(t)
            accs = [None] * 7

            def hidden(c):
                gu = _combine([_dot(lhs[i], rhs(wb_p, i, 3 * c * UR, KH)) for i in range(7)])
                return [h.astype(BF16) for h in _lhs_combos(*[_silu(z[:, :CW]) * z[:, CW:] for z in gu])]

            def down(cs, hls):
                for i in dorder:
                    l = jnp.concatenate([hl[i] for hl in hls], axis=1)
                    w = jnp.concatenate([rhs(wb_p, i, 3 * c * UR + KH, CW) for c in cs], axis=0)
                    d = _dot(l, w)
                    accs[i] = d if accs[i] is None else accs[i] + d

            pend = []
            for c in range(NC):
                hl = hidden(c)
                if not swp:
                    pend.append((c, hl))
                if len(pend) >= dgrp:
                    down(*zip(*pend))
                    pend = []
                if swp:
                    pend.append((c, hl))
            if pend:
                down(*zip(*pend))
            ys = _combine(accs)
            a = pltpu.bitcast(a_buf[...], BF16).astype(F32)
            al = _lhs_combos(a[:TH, :KH], a[:TH, KH:], a[TH:, :KH], a[TH:, KH:])
            u0 = 3 * NC * UR
            ss = _combine([_dot(al[i].astype(BF16), rhs(wb_p, i, u0, KH)) for i in range(7)])
            for n in QORDER:
                rows, cols = quad_pos(t, n)
                o_buf[rows, cols] = (x_buf[rows, cols].astype(F32) + ss[n] * _silu(ys[n])).astype(BF16)
                o_cp(t, n).start()

        x_cp(0).start()
        for cp in wa_cps(0):
            cp.start()
        off_tab[0] = 0
        wb[:, NU * UR:, :] = jnp.zeros((4, NS * SR + PR - NU * UR, KH), BF16)
        with scope("x0wait"):
            x_cp(0).wait()
        for n in range(1, x1at):
            for cp in wa_cps(n):
                cp.start()
        with scope("ln0"):
            layernorm(0, 0, keep_plain=True)
        x_cp(1).start()
        for m in range(x1at, NSUB):
            for cp in wa_cps(m):
                cp.start()
        x_cp(2).start()
        for cp in wb_cps(0):
            cp.start()
        x_cp(3).start()
        for s in range(1, min(min(v) for v in late_starts.values())):
            for cp in wb_cps(s):
                cp.start()
        phase_a0()

        def a_body(t, c):
            with scope("Await"):
                for n in (2, 3):
                    @pl.when(t + 1 == xgroups[n][0])
                    def _():
                        x_cp(n).wait()
                for s in range(NS):
                    @pl.when(t == s + 2)
                    def _():
                        for cp in wb_cps(s):
                            cp.wait()
            with scope("A"):
                phase_a(t)
            return c
        jax.lax.fori_loop(1, NT, a_body, 0)

        def b_body(t, c):
            with scope("B"):
                phase_b(t)
            return c
        jax.lax.fori_loop(0, NT, b_body, 0)
        with scope("owait"):
            for t in range(NT):
                for n in range(4):
                    o_cp(t, n).wait()

    anyspec = pl.BlockSpec(memory_space=pl.ANY)
    out = pl.pallas_call(
        kernel,
        in_specs=[anyspec] * 6,
        out_specs=anyspec,
        out_shape=jax.ShapeDtypeStruct((S, D), A_x.dtype),
        scratch_shapes=[
            pltpu.VMEM((S, D), BF16), pltpu.VMEM((TH, D), U32), pltpu.VMEM((7 * S // 4, KH), U32),
            pltpu.VMEM((4, NH, KH), BF16), pltpu.VMEM((4, NS * SR + PR, KH), BF16),
            pltpu.VMEM((7 * NH // 2, KH), U32), pltpu.VMEM((7 * NS * SR // 2, KH), U32),
            pltpu.VMEM((S // 2, 3 * D), U32),
            pltpu.VMEM((NB, TM + HALO, LANES), F32), pltpu.VMEM((NB, TM + HALO, LANES), F32),
            pltpu.VMEM((TH, D), U32), pltpu.VMEM((S, D), BF16), pltpu.SMEM((1,), jnp.int32),
            pltpu.SemaphoreType.DMA((4,)), pltpu.SemaphoreType.DMA((NSUB,)),
            pltpu.SemaphoreType.DMA((NS,)), pltpu.SemaphoreType.DMA((4 * NT,)),
        ],
        compiler_params=pltpu.CompilerParams(vmem_limit_bytes=124 * 1024 * 1024, disable_bounds_checks=True,
                                             disable_semaphore_checks=True),
    )(A_x.reshape(S, D), A_wqkv.reshape(2, KH, 3 * D), A_wo.reshape(2, KH, D),
      B_w_gate.reshape(2, KH, F), B_w_up.reshape(2, KH, F), B_w_down.reshape(2, FH, D))
    return out.reshape(B, S, D)


@jax.jit
def pallas_recurrent_scan__sliding_local_dilated__swiglu_ffn__prompt_kernel(A_x, A_wqkv, A_wo, B_x, B_w_gate, B_w_up, B_w_down):
    return build(A_x, A_wqkv, A_wo, B_x, B_w_gate, B_w_up, B_w_down)
```

```python
import contextlib
import math
import jax
import jax.numpy as jnp
import jax.experimental.pallas as pl
import jax.experimental.pallas.tpu as pltpu

F32 = jnp.float32
BF16 = jnp.bfloat16
U32 = jnp.uint32
HALO = 16
LANES = 128
QORDER = (2, 1, 3, 0)


def _butterfly(blocks):
    lane = jax.lax.broadcasted_iota(jnp.int32, blocks[0].shape, 1)
    for beta in (1, 2, 4):
        hi = (lane & (4 * beta)) != 0
        new = list(blocks)
        for j0 in range(8):
            if j0 & beta:
                continue
            j1 = j0 | beta
            new[j0] = jnp.where(hi, pltpu.roll(blocks[j1], 4 * beta, 1), blocks[j0])
            new[j1] = jnp.where(hi, blocks[j1], pltpu.roll(blocks[j0], LANES - 4 * beta, 1))
        blocks = new
    return blocks


def _opaque_zero(v):
    s = jnp.uint32(16)
    return jax.lax.shift_right_logical(jax.lax.shift_right_logical(v, s), s)


def _fzero(v):
    return pltpu.bitcast(_opaque_zero(pltpu.bitcast(v, U32)), F32)


def _silu(x):
    hx = 0.5 * x
    return hx * (1.0 + jnp.tanh(hx))


def _tree(op, xs):
    xs = list(xs)
    while len(xs) > 1:
        xs = [op(xs[i], xs[i + 1]) if i + 1 < len(xs) else xs[i] for i in range(0, len(xs), 2)]
    return xs[0]


def _lhs_combos(a11, a12, a21, a22):
    return [a11 + a22, a21 + a22, a11, a22, a11 + a12, a21 - a11, a12 - a22]


def _combine(m):
    return m[0] + m[3] - m[4] + m[6], m[2] + m[4], m[1] + m[3], m[0] - m[1] + m[2] + m[5]


def _pack(y):
    return pltpu.bitcast(y.astype(BF16), U32)


def _dot(a, b):
    return jnp.dot(a, b, preferred_element_type=F32)


def build(A_x, A_wqkv, A_wo, B_x, B_w_gate, B_w_up, B_w_down,
          subs=(128, 128, 256, 256, 256, 256, 128, 128), x1at=6, ln1=(6, 7), ln1chain=2, pchain=3, lnchain=1,
          PR=16, CG=256,  pfirst=True, rawb=True, dbg=None, zmode=1, late_starts={1: (3, 4), 2: (5,)}, uorder=(0, 1, 2), dcol=0, lnskew=0, sideat=3, morder=(0, 1, 2, 3, 4, 5, 6), wnd=0, lnp=1, dorder=(1, 3, 6, 0, 2, 4, 5), swp=False, dgrp=1, gate=False,  wchain=2, p0chain=2, scopes=False):
    scope = jax.named_scope if scopes else (lambda name: contextlib.nullcontext())
    B, S, D = A_x.shape
    F = B_w_gate.shape[1]
    H = 32
    Dh = D // H
    W, dil = 8, 2
    scale = Dh ** -0.5
    NB = D // LANES
    TM = 256
    NT = S // TM
    RC = 16
    TH = TM // 2
    TQ = TM // 4
    KH = D // 2
    FH = F // 2
    NH = 3 * D // 2
    CW = KH // 2
    NC = FH // CW
    UR = 256
    NU = 3 * NC + 2
    UPS = 4
    NS = NT - 2
    SR = UPS * UR
    assert NS * UPS >= NU and sum(subs) == NH
    NSUB = len(subs)
    PLANE = {0: 0, 2: 1, 3: 2, 5: 3, 6: 4} if rawb else {i: i for i in range(7)}
    NP = len(PLANE)
    sub_off = [sum(subs[:n]) for n in range(NSUB)]
    assert all(o // KH == (o + s - 1) // KH for o, s in zip(sub_off, subs))

    def kernel(x_hbm, wqkv_hbm, wo_hbm, wg_hbm, wu_hbm, wd_hbm, o_hbm,
               x_buf, xn0, xs_buf, wa, wb, wa_p, wb_p, qkv_raw, k_buf, v_buf, a_buf, o_buf, off_tab,
               x_sem, wa_sem, wb_sem, o_sem):
        def tile_rows(t):
            return pl.ds(pl.multiple_of(t * TM, TM), TM)

        xgroups = ((0, 1), (1, 2), (2, 4), (4, NT))

        def x_cp(n):
            rows = pl.ds(xgroups[n][0] * TM, (xgroups[n][1] - xgroups[n][0]) * TM)
            return pltpu.make_async_copy(x_hbm.at[rows, :], x_buf.at[rows, :], x_sem.at[n])

        def quad_pos(t, n):
            i, j = divmod(n, 2)
            return pl.ds(pl.multiple_of(t * TM + i * TH, TH), TH), pl.ds(j * KH, KH)

        def o_cp(t, n):
            rows, cols = quad_pos(t, n)
            return pltpu.make_async_copy(o_buf.at[rows, cols], o_hbm.at[rows, cols], o_sem.at[4 * t + n])

        def sub_pos(n):
            u, c = divmod(sub_off[n], KH)
            return pl.ds(u * KH, KH), pl.ds(c, subs[n])

        def wa_cps(n):
            rows, cols = sub_pos(n)
            return [pltpu.make_async_copy(wqkv_hbm.at[:, :, pl.ds(j * NH + sub_off[n], subs[n])],
                                          wa.at[pl.ds(2 * j, 2), rows, cols], wa_sem.at[n]) for j in range(2)]

        def wb_cps(s):
            cps = []
            u, end = s * UPS, min((s + 1) * UPS, NU)
            while u < end:
                c, part = divmod(u, 3)
                nu = 2 if (part == 0 and u + 1 < end) else 1
                rows = pl.ds(u * UR, nu * UR)
                for j in range(2):
                    dst = wb.at[pl.ds(2 * j, 2), rows, :]
                    if c == NC:
                        srcs = [(wo_hbm.at[:, pl.ds(part * UR, nu * UR), pl.ds(j * KH, KH)], dst)]
                    elif part == 2:
                        srcs = [(wd_hbm.at[:, pl.ds(c * CW, CW), pl.ds(j * KH, KH)], dst)]
                    else:
                        srcs = [(w.at[:, pl.ds(part * UR, nu * UR), pl.ds(j * FH + c * CW, CW)],
                                 wb.at[pl.ds(2 * j, 2), rows, pl.ds(n * CW, CW)])
                                for n, w in enumerate((wg_hbm, wu_hbm))]
                    cps += [pltpu.make_async_copy(a, b, wb_sem.at[s]) for a, b in srcs]
                u += nu
            return cps

        def layernorm(t, nchain, keep_plain=False, dep0=None, r_lo=0, r_hi=TH):
            deps = [] if dep0 is None else [dep0] * nchain
            g = 16
            for r in range(r_lo, r_hi, g):
                x = jnp.concatenate(
                    [x_buf[pl.ds(pl.multiple_of(t * TM + h * TH + r, g), g), :].astype(F32) for h in range(2)], axis=0)
                m = jnp.mean(x, axis=-1, keepdims=True)
                if nchain and len(deps) >= nchain:
                    m = m + pltpu.bitcast(_opaque_zero(deps[-nchain]), F32)
                xc = x - m
                var = jnp.mean(xc * xc, axis=-1, keepdims=True)
                rs = jax.lax.rsqrt(var + 1e-5)
                if gate and nchain:
                    allz = _fzero(_tree(jnp.add, [rs[q:q + 8] for q in range(0, 2 * g, 8)]))
                    rs = rs + jnp.concatenate([allz] * (2 * g // 8), axis=0)
                npiece = lnp if nchain else 1
                cw = KH // npiece
                for p in range(npiece):
                    if p > 0:
                        z = pltpu.roll(_fzero(last), 1, 1)[:, 0:1]
                        rs = rs + jnp.concatenate([z] * (2 * g // 8), axis=0)
                    cl, cr = slice(p * cw, (p + 1) * cw), slice(KH + p * cw, KH + (p + 1) * cw)
                    xl, xr = xc[:, cl] * rs, xc[:, cr] * rs
                    if keep_plain:
                        for h in range(2):
                            xn0[h * TQ + r // 2:h * TQ + (r + g) // 2, cl] = _pack(xl[h * g:(h + 1) * g])
                            xn0[h * TQ + r // 2:h * TQ + (r + g) // 2, cr] = _pack(xr[h * g:(h + 1) * g])
                    combos = _lhs_combos(xl[:g], xr[:g], xl[g:], xr[g:])
                    for n in range(7):
                        xs_buf[pl.ds(pl.multiple_of(n * (S // 4) + t * TQ + r // 2, g // 2), g // 2), cl] = _pack(combos[n])
                    last = combos[6][0:8, cw - LANES:cw]
                deps.append(pltpu.bitcast(xr[:, cw - 1:cw], U32))
            return pltpu.bitcast(last, U32)

        def prep(w, row0, nrows, c0, ncols, dst, dst_row0, nchain, dep0=None, nd=0, live=None, zmode=0):
            deps = [] if dep0 is None else [dep0] * nchain
            plane = dst.shape[0] // NP
            half0 = dst_row0 // 2
            cg = min(CG, ncols)
            for r in range(0, nrows, PR):
                src0 = row0 + r if live is None else jnp.where(live, row0 + r, NS * SR)
                rows = pl.ds(pl.multiple_of(src0, PR), PR)
                for c in range(c0, c0 + ncols, cg):
                    cols = pl.ds(c, cg)
                    b11, b21, b12, b22 = [w[s, rows, cols].astype(F32) for s in range(4)]
                    if nchain and len(deps) >= nchain:
                        z = _fzero(deps[-nchain])
                        for _ in range(max(nd, 1)):
                            z = pltpu.roll(z, 1, 1)
                        z = jnp.concatenate([jnp.concatenate([z] * (cg // LANES), axis=1)] * (PR // 8), axis=0)
                        if zmode == 0:
                            b11 = b11 + z
                            b22 = b22 + z
                        elif zmode == 2:
                            b21 = b21 + z
                    else:
                        z = None
                    outs = [b11 + b22, b11, b12 - b22, b21 - b11, b22, b11 + b12, b21 + b22]
                    if zmode == 1 and z is not None:
                        outs[6] = outs[6] + z
                    deps.append(outs[dcol * 6 if zmode == 0 else 6][PR - 8:, cg - LANES:])
                    for i in (range(7) if zmode == 0 else (6, 3, 0, 1, 2, 4, 5)):
                        if i in PLANE:
                            dst[pl.ds(pl.multiple_of(half0 + (PLANE[i] * plane + r // 2), PR // 2), PR // 2), cols] = (
                                _pack(outs[i]))
            return deps

        def rhs(dst, i, row0, nrows):
            if i not in PLANE:
                return (wa if dst is wa_p else wb)[{1: 0, 4: 3}[i], row0:row0 + nrows, :]
            p0 = PLANE[i] * (dst.shape[0] // NP) + row0 // 2
            return pltpu.bitcast(dst[p0:p0 + nrows // 2, :], BF16)

        def load_lhs(t):
            return [pltpu.bitcast(xs_buf[pl.ds(pl.multiple_of(n * (S // 4) + t * TQ, TQ), TQ), :], BF16)
                    for n in range(7)]

        def phase_a0():
            for n in range(NSUB + 1):
                if n < NSUB:
                    with scope(f"wawait{n}"):
                        for cp in wa_cps(n):
                            cp.wait()
                if n == ln1[0]:
                    with scope("x1wait"):
                        x_cp(1).wait()
                if n in ln1:
                    k = ln1.index(n)
                    layernorm(1, ln1chain, r_lo=k * TH // len(ln1), r_hi=(k + 1) * TH // len(ln1))
                if n > 0:
                    rows, cols = sub_pos(n - 1)
                    prep(wa, rows.start, KH, cols.start, cols.size, wa_p, rows.start, 0 if n == NSUB else (p0chain if subs[n] >= 256 else 2 * p0chain))
                if n < NSUB:
                    rows, cols = sub_pos(n)
                    xn = pltpu.bitcast(xn0[...], BF16)
                    for j in range(2):
                        wj = jnp.concatenate([wa[2 * j, rows, cols], wa[2 * j + 1, rows, cols]], axis=0)
                        c0 = j * NH + sub_off[n]
                        qkv_raw[0:TH, c0:c0 + subs[n]] = _pack(_dot(xn, wj))
                for s in late_starts.get(n, ()):
                    for cp in wb_cps(s):
                        cp.start()

        def phase_a(t):
            def side():
                s = jnp.where(t >= 2, t - 2, NS - 1)
                tn = jnp.minimum(t + 1, NT - 1)
                d0 = None
                if pfirst and dbg != 'noprep':
                    pd = prep(wb, s * SR, SR, 0, KH, wb_p, s * SR, wchain, nd=wnd, live=t >= 2, zmode=zmode)
                    if lnskew:
                        d0 = pltpu.bitcast(jnp.concatenate([pd[lnskew]] * 4, axis=0)[:, 0:1], U32)
                if dbg != 'noln':
                    layernorm(tn, lnchain, dep0=d0)
                if not pfirst:
                    prep(wb, s * SR, SR, 0, KH, wb_p, s * SR, wchain, nd=wnd, live=t >= 2, zmode=zmode)

            lhs = load_lhs(t)
            for u in uorder:
                if u == sideat:
                    side()
                ms = [None] * 7
                for i in morder:
                    ms[i] = _dot(lhs[i], rhs(wa_p, i, u * KH, KH))
                quads = _combine(ms)
                for n in QORDER:
                    i, j = divmod(n, 2)
                    qkv_raw[pl.ds(pl.multiple_of(t * TH + i * TQ, TQ), TQ), j * NH + u * KH:j * NH + (u + 1) * KH] = (
                        _pack(quads[n]))
            if sideat >= NH // KH:
                side()

        def permute_kv(t):
            deps = []
            for r in range(-HALO, TM, 16):
                src0 = jnp.maximum(t * TH + r // 2, 0) if r < 0 else t * TH + r // 2
                for part, dst in ((1, k_buf), (2, v_buf)):
                    src_rows = pl.ds(pl.multiple_of(src0, 8), 8)
                    blocks = [qkv_raw[src_rows, part * D + LANES * j:part * D + LANES * (j + 1)] for j in range(NB)]
                    if len(deps) >= pchain:
                        zero = _opaque_zero(deps[-pchain])
                        blocks = [b | zero for b in blocks]
                    blocks = _butterfly(blocks)
                    deps.append(blocks[NB - 1])
                    for j in range(NB):
                        dst[j, HALO + r:HALO + r + 16, :] = pltpu.bitcast(blocks[j], BF16).astype(F32)
            return _tree(jnp.bitwise_or, deps[-pchain:])

        lane = jax.lax.broadcasted_iota(jnp.int32, (RC, LANES), 1)
        odd = (lane & 1) == 1
        hi2 = (lane & 2) == 2
        rowi = jax.lax.broadcasted_iota(jnp.int32, (RC, LANES), 0)
        cexp = scale * math.log2(math.e)

        def attn_chunk(t, row0, r0, dep):
            zero = _opaque_zero(dep)
            qrows = pl.ds(pl.multiple_of(t * TH + r0 // 2, 8), RC // 2)
            qb = _butterfly([qkv_raw[qrows, LANES * j:LANES * (j + 1)] | zero for j in range(NB)])
            qs = [pltpu.bitcast(b, BF16).astype(F32) for b in qb]
            base = row0 + (HALO + r0)
            logits = []
            prev = None
            for w in range(W):
                acc = qs[0] * k_buf[0, pl.ds(base - dil * w, RC), :]
                if prev is not None:
                    acc = acc + _fzero(prev)
                for j in range(1, NB):
                    acc = acc + qs[j] * k_buf[j, pl.ds(base - dil * w, RC), :]
                prev = acc
                acc = acc + jnp.where(odd, pltpu.roll(acc, 1, 1), pltpu.roll(acc, LANES - 1, 1))
                acc = acc + jnp.where(hi2, pltpu.roll(acc, 2, 1), pltpu.roll(acc, LANES - 2, 1))
                if w > 0 and r0 < dil * w:
                    pos = rowi + (t * TM + r0 - dil * w)
                    acc = jnp.where(pos >= 0, acc, -1e9 / scale)
                logits.append(acc)
            mx = _tree(jnp.maximum, logits)
            ps = [jnp.exp2((l - mx) * cexp) for l in logits]
            den = _tree(jnp.add, ps)
            r = pl.reciprocal(den, approx=True)
            inv = r * (2.0 - den * r)
            outs = []
            prev = None
            for j in range(NB):
                o = ps[0] * v_buf[j, pl.ds(base, RC), :]
                if prev is not None:
                    o = o + _fzero(prev)
                for w in range(1, W):
                    o = o + ps[w] * v_buf[j, pl.ds(base - dil * w, RC), :]
                prev = o
                outs.append(_pack(o * inv))
            ob = _butterfly(outs)
            for j in range(NB):
                a_buf[r0 // 2:(r0 + RC) // 2, LANES * j:LANES * (j + 1)] = ob[j]
            return _tree(jnp.bitwise_or, ob)

        def phase_b(t):
            dep = permute_kv(t)
            row0 = off_tab[0]
            for r0 in range(0, TM, RC):
                dep = attn_chunk(t, row0, r0, dep)
            lhs = load_lhs(t)
            accs = [None] * 7

            def hidden(c):
                gu = _combine([_dot(lhs[i], rhs(wb_p, i, 3 * c * UR, KH)) for i in range(7)])
                return [h.astype(BF16) for h in _lhs_combos(*[_silu(z[:, :CW]) * z[:, CW:] for z in gu])]

            def down(cs, hls):
                for i in dorder:
                    l = jnp.concatenate([hl[i] for hl in hls], axis=1)
                    w = jnp.concatenate([rhs(wb_p, i, 3 * c * UR + KH, CW) for c in cs], axis=0)
                    d = _dot(l, w)
                    accs[i] = d if accs[i] is None else accs[i] + d

            pend = []
            for c in range(NC):
                hl = hidden(c)
                if not swp:
                    pend.append((c, hl))
                if len(pend) >= dgrp:
                    down(*zip(*pend))
                    pend = []
                if swp:
                    pend.append((c, hl))
            if pend:
                down(*zip(*pend))
            ys = _combine(accs)
            a = pltpu.bitcast(a_buf[...], BF16).astype(F32)
            al = _lhs_combos(a[:TH, :KH], a[:TH, KH:], a[TH:, :KH], a[TH:, KH:])
            u0 = 3 * NC * UR
            ss = _combine([_dot(al[i].astype(BF16), rhs(wb_p, i, u0, KH)) for i in range(7)])
            for n in QORDER:
                rows, cols = quad_pos(t, n)
                o_buf[rows, cols] = (x_buf[rows, cols].astype(F32) + ss[n] * _silu(ys[n])).astype(BF16)
                o_cp(t, n).start()

        x_cp(0).start()
        for cp in wa_cps(0):
            cp.start()
        off_tab[0] = 0
        wb[:, NU * UR:, :] = jnp.zeros((4, NS * SR + PR - NU * UR, KH), BF16)
        with scope("x0wait"):
            x_cp(0).wait()
        for n in range(1, x1at):
            for cp in wa_cps(n):
                cp.start()
        with scope("ln0"):
            layernorm(0, 0, keep_plain=True)
        x_cp(1).start()
        for m in range(x1at, NSUB):
            for cp in wa_cps(m):
                cp.start()
        x_cp(2).start()
        for cp in wb_cps(0):
            cp.start()
        x_cp(3).start()
        for s in range(1, min(min(v) for v in late_starts.values())):
            for cp in wb_cps(s):
                cp.start()
        phase_a0()

        def a_body(t, c):
            with scope("Await"):
                for n in (2, 3):
                    @pl.when(t + 1 == xgroups[n][0])
                    def _():
                        x_cp(n).wait()
                for s in range(NS):
                    @pl.when(t == s + 2)
                    def _():
                        for cp in wb_cps(s):
                            cp.wait()
            with scope("A"):
                phase_a(t)
            return c
        jax.lax.fori_loop(1, NT, a_body, 0)

        def b_body(t, c):
            with scope("B"):
                phase_b(t)
            return c
        jax.lax.fori_loop(0, NT, b_body, 0)
        with scope("owait"):
            for t in range(NT):
                for n in range(4):
                    o_cp(t, n).wait()

    anyspec = pl.BlockSpec(memory_space=pl.ANY)
    out = pl.pallas_call(
        kernel,
        in_specs=[anyspec] * 6,
        out_specs=anyspec,
        out_shape=jax.ShapeDtypeStruct((S, D), A_x.dtype),
        scratch_shapes=[
            pltpu.VMEM((S, D), BF16), pltpu.VMEM((TH, D), U32), pltpu.VMEM((7 * S // 4, KH), U32),
            pltpu.VMEM((4, NH, KH), BF16), pltpu.VMEM((4, NS * SR + PR, KH), BF16),
            pltpu.VMEM((NP * NH // 2, KH), U32), pltpu.VMEM((NP * NS * SR // 2, KH), U32),
            pltpu.VMEM((S // 2, 3 * D), U32),
            pltpu.VMEM((NB, TM + HALO, LANES), F32), pltpu.VMEM((NB, TM + HALO, LANES), F32),
            pltpu.VMEM((TH, D), U32), pltpu.VMEM((S, D), BF16), pltpu.SMEM((1,), jnp.int32),
            pltpu.SemaphoreType.DMA((4,)), pltpu.SemaphoreType.DMA((NSUB,)),
            pltpu.SemaphoreType.DMA((NS,)), pltpu.SemaphoreType.DMA((4 * NT,)),
        ],
        compiler_params=pltpu.CompilerParams(vmem_limit_bytes=124 * 1024 * 1024, disable_bounds_checks=True,
                                             disable_semaphore_checks=True),
    )(A_x.reshape(S, D), A_wqkv.reshape(2, KH, 3 * D), A_wo.reshape(2, KH, D),
      B_w_gate.reshape(2, KH, F), B_w_up.reshape(2, KH, F), B_w_down.reshape(2, FH, D))
    return out.reshape(B, S, D)


@jax.jit
def pallas_recurrent_scan__sliding_local_dilated__swiglu_ffn__prompt_kernel(A_x, A_wqkv, A_wo, B_x, B_w_gate, B_w_up, B_w_down):
    return build(A_x, A_wqkv, A_wo, B_x, B_w_gate, B_w_up, B_w_down)
```

```python
import math

import jax
import jax.numpy as jnp
import jax.experimental.pallas as pl
import jax.experimental.pallas.tpu as pltpu

F32 = jnp.float32
BF16 = jnp.bfloat16
U32 = jnp.uint32
LANES = 128
HALO = 16
TM = 256
RC = 16
QORDER = (2, 1, 3, 0)
PLANE = {0: 0, 2: 1, 3: 2, 5: 3, 6: 4}
RAW_SLOT = {1: 0, 4: 3}


def _butterfly(blocks):
    lane = jax.lax.broadcasted_iota(jnp.int32, blocks[0].shape, 1)
    for beta in (1, 2, 4):
        hi = (lane & (4 * beta)) != 0
        new = list(blocks)
        for j0 in range(8):
            if j0 & beta:
                continue
            j1 = j0 | beta
            new[j0] = jnp.where(hi, pltpu.roll(blocks[j1], 4 * beta, 1), blocks[j0])
            new[j1] = jnp.where(hi, blocks[j1], pltpu.roll(blocks[j0], LANES - 4 * beta, 1))
        blocks = new
    return blocks


def _opaque_zero(v):
    s = jnp.uint32(16)
    return jax.lax.shift_right_logical(jax.lax.shift_right_logical(v, s), s)


def _fzero(v):
    return pltpu.bitcast(_opaque_zero(pltpu.bitcast(v, U32)), F32)


def _silu(x):
    hx = 0.5 * x
    return hx * (1.0 + jnp.tanh(hx))


def _tree(op, xs):
    xs = list(xs)
    while len(xs) > 1:
        xs = [op(xs[i], xs[i + 1]) if i + 1 < len(xs) else xs[i] for i in range(0, len(xs), 2)]
    return xs[0]


def _lhs_combos(a11, a12, a21, a22):
    return [a11 + a22, a21 + a22, a11, a22, a11 + a12, a21 - a11, a12 - a22]


def _rhs_combos(b11, b12, b21, b22):
    return [b11 + b22, b11, b12 - b22, b21 - b11, b22, b11 + b12, b21 + b22]


def _combine(m):
    return m[0] + m[3] - m[4] + m[6], m[2] + m[4], m[1] + m[3], m[0] - m[1] + m[2] + m[5]


def _pack(y):
    return pltpu.bitcast(y.astype(BF16), U32)


def _dot(a, b):
    return jnp.dot(a, b, preferred_element_type=F32)


@jax.jit
def pallas_recurrent_scan__sliding_local_dilated__swiglu_ffn__prompt_kernel(
    A_x: jax.Array,
    A_wqkv: jax.Array,
    A_wo: jax.Array,
    B_x: jax.Array,
    B_w_gate: jax.Array,
    B_w_up: jax.Array,
    B_w_down: jax.Array,
):
    del B_x
    B, S, D = A_x.shape
    F = B_w_gate.shape[1]
    heads, window, dil = 32, 8, 2
    scale = (D // heads) ** -0.5
    NB = D // LANES
    NT = S // TM
    TH = TM // 2
    TQ = TM // 4
    KH = D // 2
    FH = F // 2
    NH = 3 * D // 2
    CW = KH // 2
    NC = FH // CW
    UR = 256
    NU = 3 * NC + 2
    UPS = 4
    NS = NT - 2
    SR = UPS * UR
    PR, CG = 16, 256
    NP = len(PLANE)
    assert B == 1 and NB == 8 and NS * UPS >= NU and dil * (window - 1) <= HALO

    subs = (128, 128, 256, 256, 256, 256, 128, 128)
    sub_off = [sum(subs[:n]) for n in range(len(subs))]
    assert sum(subs) == NH
    x1_before = 6
    ln1_rows = {6: (0, 64), 7: (64, 128)}
    prep_at = {1: (0, 4), 2: (256, 2), 3: (512, 2), 4: (768, 2), 5: (1024, 2), 7: (1280, 4)}
    late_starts = {1: (3, 4), 2: (5,)}
    xgroups = ((0, 1), (1, 2), (2, 4), (4, NT))

    def kernel(x_hbm, wqkv_hbm, wo_hbm, wg_hbm, wu_hbm, wd_hbm, o_hbm,
               x_buf, xn0, xs_buf, wa, wb, wa_p, wb_p, qkv_raw, k_buf, v_buf, a_buf, o_buf, zero_smem,
               x_sem, wa_sem, wb_sem, o_sem):
        def x_cp(n):
            rows = pl.ds(xgroups[n][0] * TM, (xgroups[n][1] - xgroups[n][0]) * TM)
            return pltpu.make_async_copy(x_hbm.at[rows, :], x_buf.at[rows, :], x_sem.at[n])

        def quad_pos(t, n):
            i, j = divmod(n, 2)
            return pl.ds(pl.multiple_of(t * TM + i * TH, TH), TH), pl.ds(j * KH, KH)

        def o_cp(t, n):
            rows, cols = quad_pos(t, n)
            return pltpu.make_async_copy(o_buf.at[rows, cols], o_hbm.at[rows, cols], o_sem.at[4 * t + n])

        def sub_pos(n):
            u, c = divmod(sub_off[n], KH)
            return pl.ds(u * KH, KH), pl.ds(c, subs[n])

        def wa_cps(n):
            rows, cols = sub_pos(n)
            return [pltpu.make_async_copy(wqkv_hbm.at[:, :, pl.ds(j * NH + sub_off[n], subs[n])],
                                          wa.at[pl.ds(2 * j, 2), rows, cols], wa_sem.at[n]) for j in range(2)]

        def wb_cps(s):
            cps = []
            u, end = s * UPS, min((s + 1) * UPS, NU)
            while u < end:
                c, part = divmod(u, 3)
                nu = 2 if (part == 0 and u + 1 < end) else 1
                rows = pl.ds(u * UR, nu * UR)
                for j in range(2):
                    dst = wb.at[pl.ds(2 * j, 2), rows, :]
                    if c == NC:
                        pairs = [(wo_hbm.at[:, pl.ds(part * UR, nu * UR), pl.ds(j * KH, KH)], dst)]
                    elif part == 2:
                        pairs = [(wd_hbm.at[:, pl.ds(c * CW, CW), pl.ds(j * KH, KH)], dst)]
                    else:
                        pairs = [(w.at[:, pl.ds(part * UR, nu * UR), pl.ds(j * FH + c * CW, CW)],
                                  wb.at[pl.ds(2 * j, 2), rows, pl.ds(n * CW, CW)])
                                 for n, w in enumerate((wg_hbm, wu_hbm))]
                    cps += [pltpu.make_async_copy(a, b, wb_sem.at[s]) for a, b in pairs]
                u += nu
            return cps

        def start(cps):
            for cp in cps:
                cp.start()

        def wait(cps):
            for cp in cps:
                cp.wait()

        def layernorm(t, nchain, keep_plain=False, r_lo=0, r_hi=TH):
            deps = []
            g = 16
            for r in range(r_lo, r_hi, g):
                x = jnp.concatenate(
                    [x_buf[pl.ds(pl.multiple_of(t * TM + h * TH + r, g), g), :].astype(F32) for h in range(2)], axis=0)
                m = jnp.mean(x, axis=-1, keepdims=True)
                if nchain and len(deps) >= nchain:
                    m = m + pltpu.bitcast(_opaque_zero(deps[-nchain]), F32)
                xc = x - m
                var = jnp.mean(xc * xc, axis=-1, keepdims=True)
                rs = jax.lax.rsqrt(var + 1e-5)
                xl, xr = xc[:, :KH] * rs, xc[:, KH:] * rs
                if keep_plain:
                    for h in range(2):
                        xn0[h * TQ + r // 2:h * TQ + (r + g) // 2, :KH] = _pack(xl[h * g:(h + 1) * g])
                        xn0[h * TQ + r // 2:h * TQ + (r + g) // 2, KH:] = _pack(xr[h * g:(h + 1) * g])
                combos = _lhs_combos(xl[:g], xr[:g], xl[g:], xr[g:])
                for n in range(7):
                    xs_buf[pl.ds(pl.multiple_of(n * (S // 4) + t * TQ + r // 2, g // 2), g // 2), :] = _pack(combos[n])
                deps.append(pltpu.bitcast(xr[:, KH - 1:KH], U32))

        def prep(w, row0, nrows, c0, ncols, dst, nchain, live=None):
            deps = []
            plane = dst.shape[0] // NP
            half0 = row0 // 2
            for r in range(0, nrows, PR):
                src0 = row0 + r if live is None else jnp.where(live, row0 + r, NS * SR)
                rows = pl.ds(pl.multiple_of(src0, PR), PR)
                for c in range(c0, c0 + ncols, CG):
                    cols = pl.ds(c, CG)
                    b11, b21, b12, b22 = [w[s, rows, cols].astype(F32) for s in range(4)]
                    z = None
                    if len(deps) >= nchain:
                        z = pltpu.roll(_fzero(deps[-nchain]), 1, 1)
                        z = jnp.concatenate([jnp.concatenate([z] * (CG // LANES), axis=1)] * (PR // 8), axis=0)
                    if z is not None and live is None:
                        b11 = b11 + z
                        b22 = b22 + z
                    outs = _rhs_combos(b11, b12, b21, b22)
                    if z is not None and live is not None:
                        outs[6] = outs[6] + z
                    deps.append(outs[0 if live is None else 6][PR - 8:, CG - LANES:])
                    for i in ((0, 2, 3, 5, 6) if live is None else (6, 3, 0, 2, 5)):
                        dst[pl.ds(pl.multiple_of(half0 + (PLANE[i] * plane + r // 2), PR // 2), PR // 2), cols] = (
                            _pack(outs[i]))

        def rhs(raw, prepared, i, row0, nrows):
            if i in RAW_SLOT:
                return raw[RAW_SLOT[i], row0:row0 + nrows, :]
            p0 = PLANE[i] * (prepared.shape[0] // NP) + row0 // 2
            return pltpu.bitcast(prepared[p0:p0 + nrows // 2, :], BF16)

        def load_lhs(t):
            return [pltpu.bitcast(xs_buf[pl.ds(pl.multiple_of(n * (S // 4) + t * TQ, TQ), TQ), :], BF16)
                    for n in range(7)]

        def startup():
            for n in range(len(subs)):
                wait(wa_cps(n))
                if n == min(ln1_rows):
                    x_cp(1).wait()
                if n in ln1_rows:
                    layernorm(1, 2, r_lo=ln1_rows[n][0], r_hi=ln1_rows[n][1])
                if n in prep_at:
                    u, c = divmod(prep_at[n][0], KH)
                    prep(wa, u * KH, KH, c, CG, wa_p, prep_at[n][1])
                rows, cols = sub_pos(n)
                xn = pltpu.bitcast(xn0[...], BF16)
                for j in range(2):
                    wj = jnp.concatenate([wa[2 * j, rows, cols], wa[2 * j + 1, rows, cols]], axis=0)
                    c0 = j * NH + sub_off[n]
                    qkv_raw[0:TH, c0:c0 + subs[n]] = _pack(_dot(xn, wj))
                for s in late_starts.get(n, ()):
                    start(wb_cps(s))

        def phase_a(t):
            lhs = load_lhs(t)
            for u in range(NH // KH):
                quads = _combine([_dot(lhs[i], rhs(wa, wa_p, i, u * KH, KH)) for i in range(7)])
                for n in QORDER:
                    i, j = divmod(n, 2)
                    qkv_raw[pl.ds(pl.multiple_of(t * TH + i * TQ, TQ), TQ), j * NH + u * KH:j * NH + (u + 1) * KH] = (
                        _pack(quads[n]))
            s = jnp.where(t >= 2, t - 2, NS - 1)
            t_next = jnp.minimum(t + 1, NT - 1)
            prep(wb, s * SR, SR, 0, KH, wb_p, 2, live=t >= 2)
            layernorm(t_next, 1)

        def permute_kv(t):
            nchain = 3
            deps = []
            for r in range(-HALO, TM, 16):
                src0 = jnp.maximum(t * TH + r // 2, 0) if r < 0 else t * TH + r // 2
                for part, dst in ((1, k_buf), (2, v_buf)):
                    src_rows = pl.ds(pl.multiple_of(src0, 8), 8)
                    blocks = [qkv_raw[src_rows, part * D + LANES * j:part * D + LANES * (j + 1)] for j in range(NB)]
                    if len(deps) >= nchain:
                        zero = _opaque_zero(deps[-nchain])
                        blocks = [b | zero for b in blocks]
                    blocks = _butterfly(blocks)
                    deps.append(blocks[NB - 1])
                    for j in range(NB):
                        dst[j, HALO + r:HALO + r + 16, :] = pltpu.bitcast(blocks[j], BF16).astype(F32)
            return _tree(jnp.bitwise_or, deps[-nchain:])

        lane = jax.lax.broadcasted_iota(jnp.int32, (RC, LANES), 1)
        odd = (lane & 1) == 1
        hi2 = (lane & 2) == 2
        rowi = jax.lax.broadcasted_iota(jnp.int32, (RC, LANES), 0)
        cexp = scale * math.log2(math.e)

        def attn_chunk(t, row0, r0, dep):
            zero = _opaque_zero(dep)
            qrows = pl.ds(pl.multiple_of(t * TH + r0 // 2, 8), RC // 2)
            qb = _butterfly([qkv_raw[qrows, LANES * j:LANES * (j + 1)] | zero for j in range(NB)])
            qs = [pltpu.bitcast(b, BF16).astype(F32) for b in qb]
            base = row0 + (HALO + r0)
            logits = []
            prev = None
            for w in range(window):
                acc = qs[0] * k_buf[0, pl.ds(base - dil * w, RC), :]
                if prev is not None:
                    acc = acc + _fzero(prev)
                for j in range(1, NB):
                    acc = acc + qs[j] * k_buf[j, pl.ds(base - dil * w, RC), :]
                prev = acc
                acc = acc + jnp.where(odd, pltpu.roll(acc, 1, 1), pltpu.roll(acc, LANES - 1, 1))
                acc = acc + jnp.where(hi2, pltpu.roll(acc, 2, 1), pltpu.roll(acc, LANES - 2, 1))
                if w > 0 and r0 < dil * w:
                    pos = rowi + (t * TM + r0 - dil * w)
                    acc = jnp.where(pos >= 0, acc, -1e9 / scale)
                logits.append(acc)
            mx = _tree(jnp.maximum, logits)
            ps = [jnp.exp2((l - mx) * cexp) for l in logits]
            den = _tree(jnp.add, ps)
            r = pl.reciprocal(den, approx=True)
            inv = r * (2.0 - den * r)
            outs = []
            prev = None
            for j in range(NB):
                o = ps[0] * v_buf[j, pl.ds(base, RC), :]
                if prev is not None:
                    o = o + _fzero(prev)
                for w in range(1, window):
                    o = o + ps[w] * v_buf[j, pl.ds(base - dil * w, RC), :]
                prev = o
                outs.append(_pack(o * inv))
            ob = _butterfly(outs)
            for j in range(NB):
                a_buf[r0 // 2:(r0 + RC) // 2, LANES * j:LANES * (j + 1)] = ob[j]
            return _tree(jnp.bitwise_or, ob)

        def phase_b(t):
            dep = permute_kv(t)
            row0 = zero_smem[0]
            for r0 in range(0, TM, RC):
                dep = attn_chunk(t, row0, r0, dep)
            lhs = load_lhs(t)
            accs = [None] * 7
            for c in range(NC):
                u0 = 3 * c * UR
                gu = _combine([_dot(lhs[i], rhs(wb, wb_p, i, u0, KH)) for i in range(7)])
                hl = [h.astype(BF16) for h in _lhs_combos(*[_silu(z[:, :CW]) * z[:, CW:] for z in gu])]
                for i in (1, 3, 6, 0, 2, 4, 5):
                    d = _dot(hl[i], rhs(wb, wb_p, i, u0 + KH, CW))
                    accs[i] = d if accs[i] is None else accs[i] + d
            ys = _combine(accs)
            a = pltpu.bitcast(a_buf[...], BF16).astype(F32)
            al = _lhs_combos(a[:TH, :KH], a[:TH, KH:], a[TH:, :KH], a[TH:, KH:])
            ss = _combine([_dot(al[i].astype(BF16), rhs(wb, wb_p, i, 3 * NC * UR, KH)) for i in range(7)])
            for n in QORDER:
                rows, cols = quad_pos(t, n)
                o_buf[rows, cols] = (x_buf[rows, cols].astype(F32) + ss[n] * _silu(ys[n])).astype(BF16)
                o_cp(t, n).start()

        x_cp(0).start()
        start(wa_cps(0))
        zero_smem[0] = 0
        wb[:, NU * UR:, :] = jnp.zeros((4, NS * SR + PR - NU * UR, KH), BF16)
        x_cp(0).wait()
        for n in range(1, x1_before):
            start(wa_cps(n))
        layernorm(0, 0, keep_plain=True)
        x_cp(1).start()
        for n in range(x1_before, len(subs)):
            start(wa_cps(n))
        x_cp(2).start()
        start(wb_cps(0))
        x_cp(3).start()
        for s in range(1, min(min(v) for v in late_starts.values())):
            start(wb_cps(s))
        startup()

        def a_body(t, carry):
            for n in (2, 3):
                pl.when(t + 1 == xgroups[n][0])(lambda n=n: x_cp(n).wait())
            for s in range(NS):
                pl.when(t == s + 2)(lambda s=s: wait(wb_cps(s)))
            phase_a(t)
            return carry
        jax.lax.fori_loop(1, NT, a_body, 0)

        def b_body(t, carry):
            phase_b(t)
            return carry
        jax.lax.fori_loop(0, NT, b_body, 0)
        for t in range(NT):
            for n in range(4):
                o_cp(t, n).wait()

    hbm = pl.BlockSpec(memory_space=pl.ANY)
    out = pl.pallas_call(
        kernel,
        in_specs=[hbm] * 6,
        out_specs=hbm,
        out_shape=jax.ShapeDtypeStruct((S, D), A_x.dtype),
        scratch_shapes=[
            pltpu.VMEM((S, D), BF16),
            pltpu.VMEM((TH, D), U32),
            pltpu.VMEM((7 * S // 4, KH), U32),
            pltpu.VMEM((4, NH, KH), BF16),
            pltpu.VMEM((4, NS * SR + PR, KH), BF16),
            pltpu.VMEM((NP * NH // 2, KH), U32),
            pltpu.VMEM((NP * NS * SR // 2, KH), U32),
            pltpu.VMEM((S // 2, 3 * D), U32),
            pltpu.VMEM((NB, TM + HALO, LANES), F32),
            pltpu.VMEM((NB, TM + HALO, LANES), F32),
            pltpu.VMEM((TH, D), U32),
            pltpu.VMEM((S, D), BF16),
            pltpu.SMEM((1,), jnp.int32),
            pltpu.SemaphoreType.DMA((len(xgroups),)),
            pltpu.SemaphoreType.DMA((len(subs),)),
            pltpu.SemaphoreType.DMA((NS,)),
            pltpu.SemaphoreType.DMA((4 * NT,)),
        ],
        compiler_params=pltpu.CompilerParams(vmem_limit_bytes=124 * 1024 * 1024, disable_bounds_checks=True,
                                             disable_semaphore_checks=True),
    )(A_x.reshape(S, D), A_wqkv.reshape(2, KH, 3 * D), A_wo.reshape(2, KH, D),
      B_w_gate.reshape(2, KH, F), B_w_up.reshape(2, KH, F), B_w_down.reshape(2, FH, D))
    return out.reshape(B, S, D)
```

```python
import math

import jax
import jax.numpy as jnp
import jax.experimental.pallas as pl
import jax.experimental.pallas.tpu as pltpu

F32 = jnp.float32
BF16 = jnp.bfloat16
U32 = jnp.uint32
LANES = 128
HALO = 16
TM = 256
RC = 16
QORDER = (2, 1, 3, 0)
PLANE = {0: 0, 2: 1, 3: 2, 5: 3, 6: 4}
RAW_SLOT = {1: 0, 4: 3}


def _butterfly(blocks):
    lane = jax.lax.broadcasted_iota(jnp.int32, blocks[0].shape, 1)
    for beta in (1, 2, 4):
        hi = (lane & (4 * beta)) != 0
        new = list(blocks)
        for j0 in range(8):
            if j0 & beta:
                continue
            j1 = j0 | beta
            new[j0] = jnp.where(hi, pltpu.roll(blocks[j1], 4 * beta, 1), blocks[j0])
            new[j1] = jnp.where(hi, blocks[j1], pltpu.roll(blocks[j0], LANES - 4 * beta, 1))
        blocks = new
    return blocks


def _opaque_zero(v):
    s = jnp.uint32(16)
    return jax.lax.shift_right_logical(jax.lax.shift_right_logical(v, s), s)


def _fzero(v):
    return pltpu.bitcast(_opaque_zero(pltpu.bitcast(v, U32)), F32)


def _silu(x):
    hx = 0.5 * x
    return hx * (1.0 + jnp.tanh(hx))


def _tree(op, xs):
    xs = list(xs)
    while len(xs) > 1:
        xs = [op(xs[i], xs[i + 1]) if i + 1 < len(xs) else xs[i] for i in range(0, len(xs), 2)]
    return xs[0]


def _lhs_combos(a11, a12, a21, a22):
    return [a11 + a22, a21 + a22, a11, a22, a11 + a12, a21 - a11, a12 - a22]


def _rhs_combos(b11, b12, b21, b22):
    return [b11 + b22, b11, b12 - b22, b21 - b11, b22, b11 + b12, b21 + b22]


def _combine(m):
    return m[0] + m[3] - m[4] + m[6], m[2] + m[4], m[1] + m[3], m[0] - m[1] + m[2] + m[5]


def _pack(y):
    return pltpu.bitcast(y.astype(BF16), U32)


def _dot(a, b):
    return jnp.dot(a, b, preferred_element_type=F32)


@jax.jit
def pallas_recurrent_scan__sliding_local_dilated__swiglu_ffn__prompt_kernel(
    A_x: jax.Array,
    A_wqkv: jax.Array,
    A_wo: jax.Array,
    B_x: jax.Array,
    B_w_gate: jax.Array,
    B_w_up: jax.Array,
    B_w_down: jax.Array,
):
    del B_x
    B, S, D = A_x.shape
    F = B_w_gate.shape[1]
    heads, window, dil = 32, 8, 2
    scale = (D // heads) ** -0.5
    NB = D // LANES
    NT = S // TM
    TH = TM // 2
    TQ = TM // 4
    KH = D // 2
    FH = F // 2
    NH = 3 * D // 2
    CW = KH // 2
    NC = FH // CW
    UR = 256
    NU = 3 * NC + 2
    UPS = 4
    NS = NT - 2
    SR = UPS * UR
    PR, CG = 16, 256
    NP = len(PLANE)
    assert B == 1 and NB == 8 and NS * UPS >= NU and dil * (window - 1) <= HALO

    subs = (128, 128, 256, 256, 256, 256, 128, 128)
    sub_off = [sum(subs[:n]) for n in range(len(subs))]
    assert sum(subs) == NH
    x1_before = 6
    ln1_rows = {6: (0, 64), 7: (64, 128)}
    prep_at = {1: (0, 4), 2: (256, 2), 3: (512, 2), 4: (768, 2), 5: (1024, 2), 7: (1280, 4)}
    late_starts = {1: (3, 4), 2: (5,)}
    xgroups = ((0, 1), (1, 2), (2, 4), (4, NT))

    def kernel(x_hbm, wqkv_hbm, wo_hbm, wg_hbm, wu_hbm, wd_hbm, o_hbm,
               x_buf, xn0, xs_buf, wa, wb, wa_p, wb_p, qkv_raw, k_buf, v_buf, a_buf, o_buf, zero_smem,
               x_sem, wa_sem, wb_sem, o_sem):
        def x_cp(n):
            rows = pl.ds(xgroups[n][0] * TM, (xgroups[n][1] - xgroups[n][0]) * TM)
            return pltpu.make_async_copy(x_hbm.at[rows, :], x_buf.at[rows, :], x_sem.at[n])

        def quad_pos(t, n):
            i, j = divmod(n, 2)
            return pl.ds(pl.multiple_of(t * TM + i * TH, TH), TH), pl.ds(j * KH, KH)

        def o_cp(t, n):
            rows, cols = quad_pos(t, n)
            return pltpu.make_async_copy(o_buf.at[rows, cols], o_hbm.at[rows, cols], o_sem.at[4 * t + n])

        def sub_pos(n):
            u, c = divmod(sub_off[n], KH)
            return pl.ds(u * KH, KH), pl.ds(c, subs[n])

        def wa_cps(n):
            rows, cols = sub_pos(n)
            return [pltpu.make_async_copy(wqkv_hbm.at[:, :, pl.ds(j * NH + sub_off[n], subs[n])],
                                          wa.at[pl.ds(2 * j, 2), rows, cols], wa_sem.at[n]) for j in range(2)]

        def wb_cps(s):
            cps = []
            u, end = s * UPS, min((s + 1) * UPS, NU)
            while u < end:
                c, part = divmod(u, 3)
                nu = 2 if (part == 0 and u + 1 < end) else 1
                rows = pl.ds(u * UR, nu * UR)
                for j in range(2):
                    dst = wb.at[pl.ds(2 * j, 2), rows, :]
                    if c == NC:
                        pairs = [(wo_hbm.at[:, pl.ds(part * UR, nu * UR), pl.ds((1 - j) * KH, KH)], dst)]
                    elif part == 2:
                        pairs = [(wd_hbm.at[:, pl.ds(c * CW, CW), pl.ds(j * KH, KH)], dst)]
                    else:
                        pairs = [(w.at[:, pl.ds(part * UR, nu * UR), pl.ds(j * FH + c * CW, CW)],
                                  wb.at[pl.ds(2 * j, 2), rows, pl.ds(n * CW, CW)])
                                 for n, w in enumerate((wg_hbm, wu_hbm))]
                    cps += [pltpu.make_async_copy(a, b, wb_sem.at[s]) for a, b in pairs]
                u += nu
            return cps

        def start(cps):
            for cp in cps:
                cp.start()

        def wait(cps):
            for cp in cps:
                cp.wait()

        def layernorm(t, nchain, keep_plain=False, r_lo=0, r_hi=TH):
            deps = []
            g = 16
            dsts = [xs_buf.at[pl.ds(pl.multiple_of(n * (S // 4) + t * TQ, TQ), TQ), :] for n in range(7)]
            for r in range(r_lo, r_hi, g):
                x = jnp.concatenate(
                    [x_buf[pl.ds(pl.multiple_of(t * TM + h * TH + r, g), g), :].astype(F32) for h in range(2)], axis=0)
                m = jnp.mean(x, axis=-1, keepdims=True)
                if nchain and len(deps) >= nchain:
                    m = m + pltpu.bitcast(_opaque_zero(deps[-nchain]), F32)
                xc = x - m
                var = jnp.mean(xc * xc, axis=-1, keepdims=True)
                rs = jax.lax.rsqrt(var + 1e-5)
                xl, xr = xc[:, :KH] * rs, xc[:, KH:] * rs
                if keep_plain:
                    for h in range(2):
                        xn0[h * TQ + r // 2:h * TQ + (r + g) // 2, :KH] = _pack(xl[h * g:(h + 1) * g])
                        xn0[h * TQ + r // 2:h * TQ + (r + g) // 2, KH:] = _pack(xr[h * g:(h + 1) * g])
                combos = _lhs_combos(xl[:g], xr[:g], xl[g:], xr[g:])
                for n in range(7):
                    dsts[n][r // 2:(r + g) // 2, :] = _pack(combos[n])
                deps.append(pltpu.bitcast(xr[:, KH - 1:KH], U32))

        def prep(w, row0, nrows, c0, ncols, dst, nchain, live=None):
            deps = []
            planes = {i: dst.at[pl.ds(pl.multiple_of(row0 // 2 + p * (dst.shape[0] // NP), 64), nrows // 2), :]
                      for i, p in PLANE.items()}
            for r in range(0, nrows, PR):
                src0 = row0 + r if live is None else jnp.where(live, row0 + r, NS * SR)
                rows = pl.ds(pl.multiple_of(src0, PR), PR)
                for c in range(c0, c0 + ncols, CG):
                    cols = pl.ds(c, CG)
                    b11, b21, b12, b22 = [w[s, rows, cols].astype(F32) for s in range(4)]
                    z = None
                    if len(deps) >= nchain:
                        z = pltpu.roll(_fzero(deps[-nchain]), 1, 1)
                        z = jnp.concatenate([jnp.concatenate([z] * (CG // LANES), axis=1)] * (PR // 8), axis=0)
                    if z is not None and live is None:
                        b11 = b11 + z
                        b22 = b22 + z
                    outs = _rhs_combos(b11, b12, b21, b22)
                    if z is not None and live is not None:
                        outs[6] = outs[6] + z
                    deps.append(outs[0 if live is None else 6][PR - 8:, CG - LANES:])
                    for i in ((0, 2, 3, 5, 6) if live is None else (6, 3, 0, 2, 5)):
                        planes[i][r // 2:(r + PR) // 2, cols] = _pack(outs[i])

        def rhs(raw, prepared, i, row0, nrows):
            if i in RAW_SLOT:
                return raw[RAW_SLOT[i], row0:row0 + nrows, :]
            p0 = PLANE[i] * (prepared.shape[0] // NP) + row0 // 2
            return pltpu.bitcast(prepared[p0:p0 + nrows // 2, :], BF16)

        def load_lhs(t):
            return [pltpu.bitcast(xs_buf[pl.ds(pl.multiple_of(n * (S // 4) + t * TQ, TQ), TQ), :], BF16)
                    for n in range(7)]

        def startup():
            for n in range(len(subs)):
                wait(wa_cps(n))
                if n == min(ln1_rows):
                    x_cp(1).wait()
                if n in ln1_rows:
                    layernorm(1, 2, r_lo=ln1_rows[n][0], r_hi=ln1_rows[n][1])
                if n in prep_at:
                    u, c = divmod(prep_at[n][0], KH)
                    prep(wa, u * KH, KH, c, CG, wa_p, prep_at[n][1])
                rows, cols = sub_pos(n)
                xn = pltpu.bitcast(xn0[...], BF16)
                for j in range(2):
                    wj = jnp.concatenate([wa[2 * j, rows, cols], wa[2 * j + 1, rows, cols]], axis=0)
                    c0 = j * NH + sub_off[n]
                    qkv_raw[0:TH, c0:c0 + subs[n]] = _pack(_dot(xn, wj))
                for s in late_starts.get(n, ()):
                    start(wb_cps(s))

        def phase_a(t):
            lhs = load_lhs(t)
            for u in range(NH // KH):
                quads = _combine([_dot(lhs[i], rhs(wa, wa_p, i, u * KH, KH)) for i in range(7)])
                for n in QORDER:
                    i, j = divmod(n, 2)
                    qkv_raw[pl.ds(pl.multiple_of(t * TH + i * TQ, TQ), TQ), j * NH + u * KH:j * NH + (u + 1) * KH] = (
                        _pack(quads[n]))
            s = jnp.where(t >= 2, t - 2, NS - 1)
            t_next = jnp.minimum(t + 1, NT - 1)
            prep(wb, s * SR, SR, 0, KH, wb_p, 2, live=t >= 2)
            layernorm(t_next, 1)

        def permute_kv(t):
            nchain = 3
            deps = []
            for r in range(-HALO, TM, 16):
                src0 = jnp.maximum(t * TH + r // 2, 0) if r < 0 else t * TH + r // 2
                for part, dst in ((1, k_buf), (2, v_buf)):
                    src_rows = pl.ds(pl.multiple_of(src0, 8), 8)
                    blocks = [qkv_raw[src_rows, part * D + LANES * j:part * D + LANES * (j + 1)] for j in range(NB)]
                    if len(deps) >= nchain:
                        zero = _opaque_zero(deps[-nchain])
                        blocks = [b | zero for b in blocks]
                    blocks = _butterfly(blocks)
                    deps.append(blocks[NB - 1])
                    for j in range(NB):
                        dst[j, HALO + r:HALO + r + 16, :] = pltpu.bitcast(blocks[j], BF16).astype(F32)
            return _tree(jnp.bitwise_or, deps[-nchain:])

        lane = jax.lax.broadcasted_iota(jnp.int32, (RC, LANES), 1)
        odd = (lane & 1) == 1
        hi2 = (lane & 2) == 2
        rowi = jax.lax.broadcasted_iota(jnp.int32, (RC, LANES), 0)
        cexp = scale * math.log2(math.e)

        def attn_chunk(t, row0, r0, dep):
            zero = _opaque_zero(dep)
            qrows = pl.ds(pl.multiple_of(t * TH + r0 // 2, 8), RC // 2)
            qb = _butterfly([qkv_raw[qrows, LANES * j:LANES * (j + 1)] | zero for j in range(NB)])
            qs = [pltpu.bitcast(b, BF16).astype(F32) for b in qb]
            base = row0 + (HALO + r0)
            logits = []
            prev = None
            for w in range(window):
                acc = qs[0] * k_buf[0, pl.ds(base - dil * w, RC), :]
                if prev is not None:
                    acc = acc + _fzero(prev)
                for j in range(1, NB):
                    acc = acc + qs[j] * k_buf[j, pl.ds(base - dil * w, RC), :]
                prev = acc
                acc = acc + jnp.where(odd, pltpu.roll(acc, 1, 1), pltpu.roll(acc, LANES - 1, 1))
                acc = acc + jnp.where(hi2, pltpu.roll(acc, 2, 1), pltpu.roll(acc, LANES - 2, 1))
                if w > 0 and r0 < dil * w:
                    pos = rowi + (t * TM + r0 - dil * w)
                    acc = jnp.where(pos >= 0, acc, -1e9 / scale)
                logits.append(acc)
            mx = _tree(jnp.maximum, logits)
            ps = [jnp.exp2((l - mx) * cexp) for l in logits]
            den = _tree(jnp.add, ps)
            r = pl.reciprocal(den, approx=True)
            inv = r * (2.0 - den * r)
            outs = []
            prev = None
            for j in range(NB):
                o = ps[0] * v_buf[j, pl.ds(base, RC), :]
                if prev is not None:
                    o = o + _fzero(prev)
                for w in range(1, window):
                    o = o + ps[w] * v_buf[j, pl.ds(base - dil * w, RC), :]
                prev = o
                outs.append(_pack(o * inv))
            ob = _butterfly(outs)
            for j in range(NB):
                a_buf[r0 // 2:(r0 + RC) // 2, LANES * j:LANES * (j + 1)] = ob[j]
            return _tree(jnp.bitwise_or, ob)

        def phase_b(t):
            dep = permute_kv(t)
            row0 = zero_smem[0]
            for r0 in range(0, TM, RC):
                dep = attn_chunk(t, row0, r0, dep)
            lhs = load_lhs(t)
            accs = [None] * 7
            for c in range(NC):
                u0 = 3 * c * UR
                gu = _combine([_dot(lhs[i], rhs(wb, wb_p, i, u0, KH)) for i in range(7)])
                hl = [h.astype(BF16) for h in _lhs_combos(*[_silu(z[:, :CW]) * z[:, CW:] for z in gu])]
                for i in (1, 3, 6, 0, 2, 4, 5):
                    d = _dot(hl[i], rhs(wb, wb_p, i, u0 + KH, CW))
                    accs[i] = d if accs[i] is None else accs[i] + d
            ys = _combine(accs)
            a = pltpu.bitcast(a_buf[...], BF16).astype(F32)
            al = _lhs_combos(a[:TH, :KH], a[:TH, KH:], a[TH:, :KH], a[TH:, KH:])
            ss = _combine([_dot(al[i].astype(BF16), rhs(wb, wb_p, i, 3 * NC * UR, KH)) for i in range(7)])
            for n in QORDER:
                rows, cols = quad_pos(t, n ^ 1)
                o_buf[rows, cols] = (x_buf[rows, cols].astype(F32) + ss[n] * _silu(ys[n ^ 1])).astype(BF16)
                o_cp(t, n ^ 1).start()

        x_cp(0).start()
        start(wa_cps(0))
        zero_smem[0] = 0
        wb[:, NU * UR:, :] = jnp.zeros((4, NS * SR + PR - NU * UR, KH), BF16)
        x_cp(0).wait()
        for n in range(1, x1_before):
            start(wa_cps(n))
        layernorm(0, 0, keep_plain=True)
        x_cp(1).start()
        for n in range(x1_before, len(subs)):
            start(wa_cps(n))
        x_cp(2).start()
        start(wb_cps(0))
        x_cp(3).start()
        for s in range(1, min(min(v) for v in late_starts.values())):
            start(wb_cps(s))
        startup()

        def a_body(t, carry):
            for n in (2, 3):
                pl.when(t + 1 == xgroups[n][0])(lambda n=n: x_cp(n).wait())
            for s in range(NS):
                pl.when(t == s + 2)(lambda s=s: wait(wb_cps(s)))
            phase_a(t)
            return carry
        jax.lax.fori_loop(1, NT, a_body, 0)

        def b_body(t, carry):
            phase_b(t)
            return carry
        jax.lax.fori_loop(0, NT, b_body, 0)
        for t in range(NT):
            for n in range(4):
                o_cp(t, n).wait()

    hbm = pl.BlockSpec(memory_space=pl.ANY)
    out = pl.pallas_call(
        kernel,
        in_specs=[hbm] * 6,
        out_specs=hbm,
        out_shape=jax.ShapeDtypeStruct((S, D), A_x.dtype),
        scratch_shapes=[
            pltpu.VMEM((S, D), BF16),
            pltpu.VMEM((TH, D), U32),
            pltpu.VMEM((7 * S // 4, KH), U32),
            pltpu.VMEM((4, NH, KH), BF16),
            pltpu.VMEM((4, NS * SR + PR, KH), BF16),
            pltpu.VMEM((NP * NH // 2, KH), U32),
            pltpu.VMEM((NP * NS * SR // 2, KH), U32),
            pltpu.VMEM((S // 2, 3 * D), U32),
            pltpu.VMEM((NB, TM + HALO, LANES), F32),
            pltpu.VMEM((NB, TM + HALO, LANES), F32),
            pltpu.VMEM((TH, D), U32),
            pltpu.VMEM((S, D), BF16),
            pltpu.SMEM((1,), jnp.int32),
            pltpu.SemaphoreType.DMA((len(xgroups),)),
            pltpu.SemaphoreType.DMA((len(subs),)),
            pltpu.SemaphoreType.DMA((NS,)),
            pltpu.SemaphoreType.DMA((4 * NT,)),
        ],
        compiler_params=pltpu.CompilerParams(vmem_limit_bytes=124 * 1024 * 1024, disable_bounds_checks=True,
                                             disable_semaphore_checks=True),
    )(A_x.reshape(S, D), A_wqkv.reshape(2, KH, 3 * D), A_wo.reshape(2, KH, D),
      B_w_gate.reshape(2, KH, F), B_w_up.reshape(2, KH, F), B_w_down.reshape(2, FH, D))
    return out.reshape(B, S, D)
```
